```python
import jax
import jax.numpy as jnp

def _softmax(x, axis=-1):
    return jax.nn.softmax(x, axis=axis)

def _gelu(x):
    return jax.nn.gelu(x, approximate=True)

def _silu(x):
    return jax.nn.silu(x)

def _sigmoid(x):
    return jax.nn.sigmoid(x)

def _layernorm(x, axis=-1, eps=1e-05):
    m = jnp.mean(x, axis=axis, keepdims=True)
    v = jnp.var(x, axis=axis, keepdims=True)
    return (x - m) / jnp.sqrt(v + eps)

def _scatter_add(tgt, idx, src, axis=0):
    return tgt.at[idx].add(src)

def _segment_sum(src, seg, n):
    return jax.ops.segment_sum(src, seg, n)

class _Rng:

    def __init__(self, key):
        self._k = key

    def _next(self):
        self._k, sub = jax.random.split(self._k)
        return sub

    def normal(self, shape):
        return jax.random.normal(self._next(), shape, dtype=jnp.bfloat16)

    def randint(self, lo, hi, shape):
        return jax.random.randint(self._next(), shape, lo, hi, dtype=jnp.int32)

    def uniform(self, shape, lo=0.0, hi=1.0):
        return jax.random.uniform(self._next(), shape, jnp.bfloat16, lo, hi)

    def permutation(self, n):
        return jax.random.permutation(self._next(), n)
kernel_name = 'adaLN_cond__grouped_kv_mqa__mixer_token_mlp__prompt'

def _fwd_setup_inputs():
    _rng = _Rng(jax.random.key(int.from_bytes(__import__("os").urandom(4), "little")))
    _w = lambda a: (lambda t: t.astype(jnp.bfloat16) if jnp.issubdtype(t.dtype, jnp.floating) else t)(jnp.asarray(a))

    def _A_setup():
        B, S, D, H = (1, 2048, 512, 32)
        Dh = D // H
        return {'x': _w((lambda *s: _rng.normal(s) * 0.05)(B, S, D)), 'wq': _w((lambda *s: _rng.normal(s) * 0.05)(D, H * Dh)), 'wk': _w((lambda *s: _rng.normal(s) * 0.05)(D, Dh)), 'wv': _w((lambda *s: _rng.normal(s) * 0.05)(D, Dh)), 'wo': _w((lambda *s: _rng.normal(s) * 0.05)(H * Dh, D))}
    _A_in = _A_setup()

    def _B_setup():
        B, S, D, F = (1, 2048, 512, 1376)
        return {'x': _w((lambda *s: _rng.normal(s) * 0.05)(B, S, D)), 'w1': _w((lambda *s: _rng.normal(s) * 0.05)(S, F) * S ** (-0.5)), 'b1': _w((lambda *s: _rng.normal(s) * 0.05)(F) * 0.02), 'w2': _w((lambda *s: _rng.normal(s) * 0.05)(F, S) * F ** (-0.5)), 'b2': _w((lambda *s: _rng.normal(s) * 0.05)(S) * 0.02)}
    _B_in = _B_setup()
    return {'A_x': _A_in['x'], 'A_wq': _A_in['wq'], 'A_wk': _A_in['wk'], 'A_wv': _A_in['wv'], 'A_wo': _A_in['wo'], 'B_x': _B_in['x'], 'B_w1': _B_in['w1'], 'B_b1': _B_in['b1'], 'B_w2': _B_in['w2'], 'B_b2': _B_in['b2'], 'c': _w((lambda *s: _rng.normal(s) * 0.05)(1, 512)), 'w_mod': _w((lambda *s: _rng.normal(s) * 0.05)(512, 6 * 512) * 512 ** (-0.5))}

def _fwd_reference(A_x, A_wq, A_wk, A_wv, A_wo, B_x, B_w1, B_b1, B_w2, B_b2, c, w_mod):

    def _A_ref(x, wq, wk, wv, wo):
        B, S, D = x.shape
        H = 32
        Dh = D // H
        q = (lambda x, *d: x.transpose(*d))((x @ wq).reshape(B, S, H, Dh), 0, 2, 1, 3)
        k = x @ wk
        v = x @ wv
        scores = jnp.einsum('bhqd,bkd->bhqk', q, k) * Dh ** (-0.5)
        p = _softmax(scores, axis=-1)
        o = jnp.einsum('bhqk,bkd->bhqd', p, v)
        return (lambda x, *d: x.transpose(*d))(o, 0, 2, 1, 3).reshape(B, S, H * Dh) @ wo

    def _B_ref(x, w1, b1, w2, b2):
        B, S, D = x.shape
        h = _layernorm(x, axis=-1)
        u = jnp.einsum('bsd,sf->bdf', h, w1) + b1
        u = _gelu(u)
        y = jnp.einsum('bdf,fs->bds', u, w2) + b2
        return (lambda x, *d: x.transpose(*d))(y, 0, 2, 1)
    x = A_x
    mod = (_silu(c) @ w_mod).reshape(c.shape[0], 6, 1, -1)
    sa, ca, ga, sb, cb, gb = (mod[:, 0].copy(), mod[:, 1].copy(), mod[:, 2].copy(), mod[:, 3].copy(), mod[:, 4].copy(), mod[:, 5].copy())
    h = _layernorm(x, axis=-1) * (1 + ca) + sa
    x = x + ga * _A_ref(h, A_wq, A_wk, A_wv, A_wo)
    h = _layernorm(x, axis=-1) * (1 + cb) + sb
    x = x + gb * _B_ref(h, B_w1, B_b1, B_w2, B_b2)
    return x

def setup_inputs():
    _inp = _fwd_setup_inputs()
    _gk = jax.random.fold_in(jax.random.key(int.from_bytes(__import__("os").urandom(4), "little")), 2 ** 31 - 1)
    _shapes = [[1, 2048, 512]]
    _dtypes = ['bfloat16']
    _gks = jax.random.split(_gk, len(_shapes))
    _gs = [jax.random.normal(k, s, dtype=jnp.dtype(d)) * 0.05 for k, s, d in zip(_gks, _shapes, _dtypes)]
    _inp['grad_out'] = _gs[0]
    return _inp

def reference(A_x, A_wq, A_wk, A_wv, A_wo, B_w1, B_b1, B_w2, B_b2, c, w_mod, B_x, grad_out):
    _const = dict(B_x=B_x)

    def _f(*_d):
        return _fwd_reference(**{'A_x': _d[0], 'A_wq': _d[1], 'A_wk': _d[2], 'A_wv': _d[3], 'A_wo': _d[4], 'B_w1': _d[5], 'B_b1': _d[6], 'B_w2': _d[7], 'B_b2': _d[8], 'c': _d[9], 'w_mod': _d[10], **_const})
    _out, _vjp = jax.vjp(_f, A_x, A_wq, A_wk, A_wv, A_wo, B_w1, B_b1, B_w2, B_b2, c, w_mod)
    _grads = _vjp(grad_out)
    _out0 = jnp.asarray(_out)
    return (_out0, *[jnp.asarray(_g) for _g in _grads])
```

```python
import contextlib

import jax
import jax.numpy as jnp
from jax import lax
import jax.experimental.pallas as pl
import jax.experimental.pallas.tpu as pltpu

S, D, H, DH, F = 2048, 512, 32, 16, 1376
EPS = 1e-5
LOG2E = 1.4426950408889634
LN2 = 0.6931471805599453
QSCALE = 0.25 * LOG2E
C0 = 0.7978845608028654
C1 = 0.044715

LT = 128
NLT = S // LT
W = 256
NQ = S // W
NT = H * NQ
NIT = NT // 4
KC_F = 512
SUB_F = 256
KC_B = 256
SUB_B = 64
MB = 128
RB = 64
AR = 32
NFC = F // 128
FT = F % 128
SAFE_BOUND = 40.0

_PROFILE = False


def _scope(name):
    return jax.named_scope(name) if _PROFILE else contextlib.nullcontext()


F32 = jnp.float32
BF16 = jnp.bfloat16
U32 = jnp.uint32
NT_DIMS = (((1,), (1,)), ((), ()))


def _dot(a, b):
    return jnp.dot(a, b, preferred_element_type=F32)


def _dot_nt(a, b):
    return lax.dot_general(a, b, NT_DIMS, preferred_element_type=F32)


def _tile(i, n):
    return pl.ds(pl.multiple_of(i * n, n), n)


def _pk(x):
    return pltpu.bitcast(x, U32)


def _up(x):
    return pltpu.bitcast(x, BF16)


def _pr(m, n):
    return slice(m // 2, (m + n) // 2)


def _split3(x):
    hi = x.astype(BF16).astype(F32)
    r = x - hi
    mid = r.astype(BF16).astype(F32)
    lo = (r - mid).astype(BF16).astype(F32)
    return hi, mid, lo


def _rows16(vals, shape, axis):
    row = lax.broadcasted_iota(jnp.int32, shape, axis)
    blk = jnp.zeros(shape, F32)
    for k, v in enumerate(vals):
        blk = jnp.where(row == k, v, blk)
    return blk.astype(BF16)


def _bsum(x):
    return x.reshape(x.shape[0] // 8, 8, x.shape[1]).sum(axis=0)


def _fin(s8):
    return jnp.sum(s8, axis=0, keepdims=True)


def _moments(s1, s2, c):
    d = _fin(s1) * (1.0 / D)
    var = jnp.maximum(_fin(s2) * (1.0 / D) - d * d, 0.0)
    return c + d, lax.rsqrt(var + EPS)


def _row_of(acc):
    return jnp.sum(acc.T, axis=0, keepdims=True)


def _lanes(t):
    return pl.ds(pl.multiple_of((t % NQ) * W, W), W)


def _blocks(n, step):
    return [slice(m, min(m + step, n)) for m in range(0, n, step)]


def _kernel(
    x_hbm, wq_ref, wk_ref, wv_ref, wo_ref, w1_hbm, b1_ref, w2_hbm, b2_ref, c_ref, wmod_hbm, go_hbm,
    out_hbm, dx_hbm, dwq_ref, dwk_ref, dwv_ref, dwo_ref, dw1_hbm, db1_ref, dw2_hbm, db2_ref, dc_ref, dwmod_hbm,
    p_hbm,
    pres, QA, DOA, KA, VA, KT, VT, x_raw, go_raw, w1_v, w2_v, oT, h1T, goT, dxT, st, modc, modrow, acc_s,
    woT_s, wqT_s, b1v, b2v, dmod_s,
    sem_in, sem_out, sem_p,
):
    V = pltpu.VMEM
    cp_x = pltpu.make_async_copy(x_hbm, x_raw, sem_in.at[0])
    cp_w1 = pltpu.make_async_copy(w1_hbm, w1_v, sem_in.at[2])
    cp_w2 = pltpu.make_async_copy(w2_hbm, w2_v, sem_in.at[3])
    cp_go = pltpu.make_async_copy(go_hbm, go_raw, sem_in.at[4])

    def cp_out(i):
        return pltpu.make_async_copy(go_raw.at[_tile(i, LT), :], out_hbm.at[_tile(i, LT), :], sem_out.at[0])

    def cp_dw2(i):
        return pltpu.make_async_copy(w2_v.at[:, _tile(i, LT)], dw2_hbm.at[:, _tile(i, LT)], sem_out.at[1])

    def cp_dw1(i):
        return pltpu.make_async_copy(w1_v.at[:, _tile(i, LT)], dw1_hbm.at[:, _tile(i, LT)], sem_out.at[2])

    def cp_dx(i):
        return pltpu.make_async_copy(x_raw.at[_tile(i, LT), :], dx_hbm.at[_tile(i, LT), :], sem_out.at[3])

    cvec = c_ref[...].astype(F32)
    csig = jax.nn.sigmoid(cvec)
    sc = cvec * csig
    wkvT = jnp.concatenate([wk_ref[...], wv_ref[...]], axis=0)
    z8 = jnp.zeros((8, LT), F32)
    inv_d = 1.0 / D

    def pipeline(n, mm, ew, bufs):
        mm(0, bufs[0])

        def body(j, carry):
            i = 2 * j
            ew(i, bufs[0])
            mm(i + 1, bufs[1])
            ew(i + 1, bufs[1])
            mm(i + 2, bufs[0])
            return carry
        lax.fori_loop(0, n // 2 - 1, body, 0)
        ew(n - 2, bufs[0])
        mm(n - 1, bufs[1])
        ew(n - 1, bufs[1])

    def scope1(wmod_v, kv_s, xb, h1a, h1b, qn_s, pb0, hb, l0, l1):
        def mod_parts(lo, hi):
            mod = _dot(jnp.broadcast_to(sc, (16, D)).astype(BF16), wmod_v[:, lo * D:hi * D])[0:1]
            modrow[:, lo * D:hi * D] = mod
            for r in range(lo, hi):
                m_r = mod[:, (r - lo) * D:(r - lo + 1) * D]
                if r in (1, 4):
                    m_r = m_r + 1.0
                modc[r] = jnp.broadcast_to(m_r, (LT, D)).T

        with _scope("P1"):
            cp_wma = pltpu.make_async_copy(wmod_hbm.at[:, 0:2 * D], wmod_v.at[:, 0:2 * D], sem_in.at[1])
            cp_wmb = pltpu.make_async_copy(wmod_hbm.at[:, 2 * D:6 * D], wmod_v.at[:, 2 * D:6 * D], sem_in.at[5])
            cp_x.start()
            cp_wma.start()
            b1v[...] = b1_ref[...].astype(F32).reshape(1, F)
            b2v[...] = b2_ref[...].astype(F32).reshape(1, S)
            wqT_s[...] = _pk(wq_ref[...].T)
            woT_s[...] = _pk(wo_ref[...].T)
            qn_s[...] = jnp.zeros(qn_s.shape, F32)
            cp_wma.wait()
            mod_parts(0, 2)

        with _scope("P2"):
            cp_x.wait()
            cp_wmb.start()
            cp_go.start()
            cp_w1.start()

            def ln1_chunk(i, hbuf):
                tl = _tile(i, LT)
                for rs in _blocks(D, LT):
                    xb[rs, :] = x_raw[tl, rs].T.astype(F32)
                c = xb[0:1, :]
                s1 = s2 = z8
                for rs in _blocks(D, RB):
                    d = xb[rs, :] - c
                    s1 = s1 + _bsum(d)
                    s2 = s2 + _bsum(d * d)
                mu, r = _moments(s1, s2, c)
                st[0:1, tl] = mu
                st[1:2, tl] = r
                for rs in _blocks(D, RB):
                    h1 = _pk((((xb[rs, :] - mu) * r) * modc[1, rs] + modc[0, rs]).astype(BF16))
                    hbuf[_pr(rs.start, RB), :] = h1
                    h1T[_pr(rs.start, RB), tl] = h1

            def proj_chunk(i, hbuf):
                tl = _tile(i, LT)
                h1 = _up(hbuf[...])
                kv_s[:, tl] = _dot(wkvT, h1)
                for m in range(0, D, 256):
                    q = (_dot(_up(wqT_s[_pr(m, 256), :]), h1) * QSCALE).astype(BF16)
                    q3 = q.reshape(256 // DH, DH, LT)
                    hs = slice(m // DH, (m + 256) // DH)
                    QA[hs, 0:DH, tl] = q3
                    QA[hs, DH:AR, tl] = jnp.zeros((256 // DH, AR - DH, LT), BF16)
                    qf = q3.astype(F32)
                    qn_s[...] = jnp.maximum(qn_s[...], jnp.max(jnp.sum(qf * qf, axis=1), axis=0, keepdims=True))

            pipeline(NLT, ln1_chunk, proj_chunk, (h1a, h1b))

        with _scope("P3"):
            kvT = kv_s[...]
            kTb = kvT[0:DH].astype(BF16)
            vTb = kvT[DH:2 * DH].astype(BF16)
            KT[...] = kTb
            VT[...] = vTb
            rows = lax.broadcasted_iota(jnp.int32, (LT - DH, S), 0)
            tail = jnp.where(rows < 3, 1.0, 0.0).astype(BF16)
            ka_t = jnp.concatenate([kTb, tail], axis=0)
            va_t = jnp.concatenate([vTb, tail], axis=0)
            for j in range(NLT):
                KA[_pr(j * LT, LT), :] = _pk(ka_t[:, j * LT:(j + 1) * LT].T)
                VA[_pr(j * LT, LT), :] = _pk(va_t[:, j * LT:(j + 1) * LT].T)

            kf = kTb.astype(F32)
            kn2 = jnp.max(jnp.sum(kf * kf, axis=0, keepdims=True))
            bound2 = jnp.max(qn_s[...]) * kn2
            vmax = jnp.max(jnp.abs(vTb.astype(F32)))
            safe = jnp.logical_and(bound2 <= SAFE_BOUND * SAFE_BOUND, vmax <= 1e15)

            cp_wmb.wait()
            mod_parts(2, 6)
            cp_go.wait()

        def keys(ref, lo, n):
            return _up(ref[_pr(lo, n), :])[:, 0:AR]

        with _scope("P4max"):
            @pl.when(jnp.logical_not(safe))
            def _():
                def pmax(t, carry):
                    h = t // NQ
                    q = QA[h, :, _lanes(t)]
                    m = None
                    for lo in range(0, S, KC_F):
                        mc = jnp.max(_dot(keys(KA, lo, KC_F), q), axis=0, keepdims=True)
                        m = mc if m is None else jnp.maximum(m, mc)
                    hi, mid, lo_ = _split3(m)
                    QA[h, DH:AR, _lanes(t)] = _rows16((-hi, -mid, -lo_), (AR - DH, W), 0)
                    return carry
                lax.fori_loop(0, NT, pmax, 0)

        def p_out(idx):
            return pltpu.make_async_copy(hb.at[idx % 4], p_hbm.at[idx], sem_p.at[idx % 4])

        def fwd_step(t_next, pn, ln, t_cur, pc, lc):
            q = QA[t_next // NQ, :, _lanes(t_next)]
            lacc = jnp.zeros((32, W), F32)
            o = jnp.zeros((DH, W), F32)
            for c in range(S // KC_F):
                for lo in range(c * KC_F, (c + 1) * KC_F, SUB_F):
                    p = jnp.exp2(_dot(keys(KA, lo, SUB_F), q))
                    pn[_pr(lo, SUB_F), :] = _pk(p.astype(BF16))
                    lacc = lacc + p.reshape(SUB_F // 32, 32, W).sum(axis=0)
                if t_cur is not None:
                    for lo in range(c * KC_F, (c + 1) * KC_F, 128):
                        o = o + _dot(VT[:, lo:lo + 128], _up(pc[_pr(lo, 128), :]))
            lnew = lacc.sum(axis=0, keepdims=True)
            if t_cur is not None:
                hc = t_cur // NQ
                linv = 1.0 / lc[...]
                oT[pl.ds(pl.multiple_of(hc * (DH // 2), DH // 2), DH // 2), _lanes(t_cur)] = _pk(
                    (o * linv).astype(BF16))
                sh = QA[hc, DH:AR, _lanes(t_cur)].astype(F32)
                hi, mid, lo = _split3(linv)
                QA[hc, DH:AR, _lanes(t_cur)] = _rows16(
                    (sh[0:1], sh[1:2], sh[2:3], hi, mid, lo), (AR - DH, W), 0)
            ln[...] = lnew

        with _scope("P4"):
            fwd_step(0, pb0, l0, None, None, None)

            def fwd_body(it, carry):
                t = 4 * it
                pv = pres.at[it]
                ha = hb.at[(2 * it) % 4]
                hc = hb.at[(2 * it + 1) % 4]

                @pl.when(it >= 2)
                def _():
                    p_out(2 * it - 4).wait()
                    p_out(2 * it - 3).wait()
                goT[_tile(it % 4, LT // 2), _tile(it // 4, LT)] = _pk(
                    go_raw[_tile(it // 4, LT), _tile(it % 4, LT)].T)
                fwd_step(t + 1, ha, l1, t, pb0, l0)
                p_out(2 * it).start()
                fwd_step(t + 2, pv, l0, t + 1, ha, l1)
                fwd_step(t + 3, hc, l1, t + 2, pv, l0)
                p_out(2 * it + 1).start()
                fwd_step(jnp.minimum(t + 4, NT - 1), pb0, l0, t + 3, hc, l1)
                return carry
            lax.fori_loop(0, NIT, fwd_body, 0)
            cp_w2.start()
            for k in range(4):
                p_out(2 * NIT - 4 + k).wait()

    pl.run_scoped(scope1, V((D, 6 * D), BF16), V((2 * DH, S), F32), V((D, LT), F32),
                  V((D // 2, LT), U32), V((D // 2, LT), U32), V((1, LT), F32),
                  V((S // 2, W), U32), V((4, S // 2, W), U32),
                  V((1, W), F32), V((1, W), F32))

    def scope2(x1T, h3T, g_s, gT_s, du_s, duT_s, dx1b, dgbuf, wog, m_acc, ta, tb, tc, td):
        def a_mm(i, abuf):
            och = _up(oT[:, _tile(i, LT)])
            for m in range(0, D, 256):
                abuf[m:m + 256, :] = _dot(_up(woT_s[_pr(m, 256), :]), och)

        def dg_mm(sl):
            w2r = w2_v[sl, :]
            for m in range(0, D, 256):
                dgbuf[m:m + 256, sl] = _dot_nt(_up(goT[_pr(m, 256), :]), w2r)

        def p5_ew(i, abuf):
            tl = _tile(i, LT)
            for rs in _blocks(D, LT):
                x1T[rs, tl] = x_raw[tl, rs].T.astype(F32) + modc[2, rs] * abuf[rs, :]
            c = x1T[0:1, tl]
            s1 = s2 = z8
            for rs in _blocks(D, RB):
                d = x1T[rs, tl] - c
                s1 = s1 + _bsum(d)
                s2 = s2 + _bsum(d * d)
            mu2, r2 = _moments(s1, s2, c)

            def h2_of(rs):
                return ((x1T[rs, tl] - mu2) * r2) * modc[4, rs] + modc[3, rs]
            c3 = h2_of(slice(0, 8))[0:1]
            s1 = s2 = z8
            for rs in _blocks(D, RB):
                d = h2_of(rs) - c3
                s1 = s1 + _bsum(d)
                s2 = s2 + _bsum(d * d)
            mu3, r3 = _moments(s1, s2, c3)
            st[2:3, tl] = mu2
            st[3:4, tl] = r2
            st[4:5, tl] = mu3
            st[5:6, tl] = r3
            for rs in _blocks(D, RB):
                h3T[_pr(rs.start, RB), tl] = _pk(((h2_of(rs) - mu3) * r3).astype(BF16))

        with _scope("P5"):
            a_mm(0, ta)

            def p5a(j, carry):
                i = 2 * j
                p5_ew(i, ta)
                a_mm(i + 1, tb)
                p5_ew(i + 1, tb)
                a_mm(i + 2, ta)
                return carry
            lax.fori_loop(0, 2, p5a, 0)
            p5_ew(4, ta)
            a_mm(5, tb)
            cp_w2.wait()
            p5_ew(5, tb)
            a_mm(6, ta)
            dg_mm(slice(NFC * 128, F))

            def p5b(j, carry):
                i = 6 + 2 * j
                p5_ew(i, ta)
                a_mm(i + 1, tb)
                dg_mm(_tile(2 * j, 128))
                p5_ew(i + 1, tb)
                a_mm(jnp.minimum(i + 2, NLT - 1), ta)
                dg_mm(_tile(2 * j + 1, 128))
                return carry
            lax.fori_loop(0, NFC // 2, p5b, 0)

        def u_mm(sl, n, ubuf):
            w1r = w1_v[sl, :]
            for m in range(0, D, 256):
                ubuf[m:m + 256, 0:n] = _dot_nt(_up(h3T[_pr(m, 256), :]), w1r)

        def f_ew(sl, sl2, n, ubuf):
            b1r = b1v[:, sl]
            sdb = jnp.zeros((8, n), F32)
            for rs in _blocks(D, LT):
                gb = modc[5, rs, 0:n]
                u = ubuf[rs, 0:n] + b1r
                u2 = u * u
                t = jnp.tanh(C0 * u * (1.0 + C1 * u2))
                hp = 0.5 * (1.0 + t)
                g = u * hp
                du = (dgbuf[rs, sl] * gb) * (hp + 0.5 * u * (1.0 - t * t) * C0 * (1.0 + 3.0 * C1 * u2))
                dub = du.astype(BF16)
                g_s[_pr(rs.start, LT), sl] = _pk(g.astype(BF16))
                du_s[_pr(rs.start, LT), sl] = _pk(dub)
                gT_s[sl2, rs] = _pk((g * gb).astype(BF16).T)
                duT_s[sl2, rs] = _pk(dub.T)
                sdb = sdb + _bsum(du)
            db1_ref[:, sl] = _fin(sdb).astype(BF16)

        with _scope("P6"):
            cp_w1.wait()
            u_mm(slice(0, 128), 128, ta)

            def p6(j, carry):
                i = 2 * j
                f_ew(_tile(i, 128), _tile(i, 64), 128, ta)
                u_mm(_tile(i + 1, 128), 128, tb)
                f_ew(_tile(i + 1, 128), _tile(i + 1, 64), 128, tb)
                u_mm(_tile(i + 2, 128), 128, ta)
                return carry
            lax.fori_loop(0, NFC // 2 - 1, p6, 0)
            i8, i9 = NFC - 2, NFC - 1
            f_ew(slice(i8 * 128, i9 * 128), slice(i8 * 64, i9 * 64), 128, ta)
            u_mm(slice(i9 * 128, NFC * 128), 128, tb)
            f_ew(slice(i9 * 128, NFC * 128), slice(i9 * 64, NFC * 64), 128, tb)
            u_mm(slice(NFC * 128, F), FT, ta)
            f_ew(slice(NFC * 128, F), slice(NFC * 64, F // 2), FT, ta)

        def p7_mm(i, bufs):
            yb, hb_ = bufs
            tl = _tile(i, LT)
            w2c = w2_v[:, tl]
            w1c = w1_v[:, tl]
            for m in range(0, D, MB):
                yb[m:m + MB, :] = _dot(_up(g_s[_pr(m, MB), :]), w2c)
            for m in range(0, D, MB):
                hb_[m:m + MB, :] = _dot(_up(du_s[_pr(m, MB), :]), w1c)
            goc = _up(goT[:, tl])
            h3c = _up(h3T[:, tl])
            for rs in _blocks(F, MB):
                w2_v[rs, tl] = _dot(_up(gT_s[_pr(rs.start, rs.stop - rs.start), :]), goc).astype(BF16)
            for rs in _blocks(F, MB):
                w1_v[rs, tl] = _dot(_up(duT_s[_pr(rs.start, rs.stop - rs.start), :]), h3c).astype(BF16)
            cp_dw2(i).start()
            cp_dw1(i).start()

        def p7_ew(i, bufs):
            yb, hb_ = bufs
            tl = _tile(i, LT)
            b2r = b2v[:, tl]
            mu2, r2, mu3, r3 = st[2:3, tl], st[3:4, tl], st[4:5, tl], st[5:6, tl]
            for rs in _blocks(D, LT):
                go_raw[tl, rs] = (x1T[rs, tl] + modc[5, rs] * (yb[rs, :] + b2r)).astype(BF16).T
            cp_out(i).start()

            def norms(rs):
                n2 = (x1T[rs, tl] - mu2) * r2
                h3 = (n2 * modc[4, rs] + modc[3, rs] - mu3) * r3
                return n2, h3

            def dx2_of(rs):
                return _up(goT[_pr(rs.start, RB), tl]).astype(F32)

            s1 = s2 = sdb = z8
            for rs in _blocks(D, RB):
                dx2 = dx2_of(rs)
                acc_s[5, rs] += dx2 * (yb[rs, :] + b2r)
                sdb = sdb + _bsum(modc[5, rs] * dx2)
                _, h3 = norms(rs)
                dh3 = hb_[rs, :]
                s1 = s1 + _bsum(dh3)
                s2 = s2 + _bsum(dh3 * h3)
            db2_ref[:, tl] = _fin(sdb).astype(BF16)
            m1 = _fin(s1) * inv_d
            m2 = _fin(s2) * inv_d
            s3 = s4 = z8
            for rs in _blocks(D, RB):
                n2, h3 = norms(rs)
                dh2 = r3 * (hb_[rs, :] - m1 - h3 * m2)
                acc_s[4, rs] += dh2 * n2
                acc_s[3, rs] += dh2
                dn2 = dh2 * modc[4, rs]
                hb_[rs, :] = dn2
                s3 = s3 + _bsum(dn2)
                s4 = s4 + _bsum(dn2 * n2)
            m3 = _fin(s3) * inv_d
            m4 = _fin(s4) * inv_d
            for rs in _blocks(D, RB):
                n2 = (x1T[rs, tl] - mu2) * r2
                dx1 = dx2_of(rs) + r2 * (hb_[rs, :] - m3 - n2 * m4)
                dxT[rs, tl] = dx1
                dx1b[_pr(rs.start, RB), tl] = _pk(dx1.astype(BF16))

        with _scope("P7"):
            acc_s[...] = jnp.zeros(acc_s.shape, F32)
            pipeline(NLT, p7_mm, p7_ew, ((ta, tb), (tc, td)))

        def p8_mm(i, dbuf_):
            tl = _tile(i, LT)
            dxc = _up(dx1b[:, tl])
            for m in range(0, D, 256):
                dbuf_[m:m + 256, :] = _dot(_up(wog[_pr(m, 256), :]), dxc)
            for m in range(0, D, 256):
                m_acc[m:m + 256, :] += _dot_nt(_up(oT[_pr(m, 256), tl]), dxc)

        def p8_ew(i, dbuf_):
            tl = _tile(i, LT)
            hpb = RB // DH
            for rs in _blocks(D, RB):
                hs = slice(rs.start // DH, rs.stop // DH)
                li = QA[hs, DH:AR, tl].astype(F32)
                linv = li[:, 3:4] + li[:, 4:5] + li[:, 5:6]
                dos = (dbuf_[rs, :].reshape(hpb, DH, LT) * linv).astype(BF16)
                of = _up(oT[_pr(rs.start, RB), tl]).astype(F32).reshape(hpb, DH, LT)
                delta = jnp.sum(dos.astype(F32) * of, axis=1, keepdims=True)
                hi, mid, lo = _split3(delta)
                DOA[hs, 0:DH, tl] = dos
                DOA[hs, DH:AR, tl] = _rows16((-hi, -mid, -lo), (hpb, AR - DH, LT), 1)

        with _scope("P8"):
            garow = modrow[:, 2 * D:3 * D]
            wof = wo_ref[...].astype(F32)
            wog[...] = _pk((wof * garow).astype(BF16))
            m_acc[...] = jnp.zeros(m_acc.shape, F32)
            pipeline(NLT, p8_mm, p8_ew, (ta, tb))
            m_od = m_acc[...]
            dwo_ref[...] = (m_od * garow).astype(BF16)
            dmod_s[:, 2 * D:3 * D] = jnp.sum(m_od * wof, axis=0, keepdims=True)
            for r in (3, 4, 5):
                dmod_s[:, r * D:(r + 1) * D] = _row_of(acc_s[r])

    pl.run_scoped(scope2, V((D, S), F32), V((D // 2, S), U32), V((D // 2, F), U32),
                  V((F // 2, D), U32), V((D // 2, F), U32), V((F // 2, D), U32), V((D // 2, S), U32),
                  V((D, F), F32), V((D // 2, D), U32), V((D, D), F32),
                  V((D, LT), F32), V((D, LT), F32), V((D, LT), F32), V((D, LT), F32))

    def scope3(pb0, hb, db0, db1, dqT, dkT, dvT, dkv_s, wmod_v, dwm_st, dwq_acc, wqp, ta, tb, nb):
        cp_wmod = pltpu.make_async_copy(wmod_hbm, wmod_v, sem_in.at[1])
        cp_dwm_b = pltpu.make_async_copy(dwm_st.at[:, 2 * D:6 * D], dwmod_hbm.at[:, 2 * D:6 * D], sem_out.at[4])
        cp_dwm_a = pltpu.make_async_copy(dwm_st.at[:, 0:2 * D], dwmod_hbm.at[:, 0:2 * D], sem_out.at[5])
        sc_col = jnp.broadcast_to(sc, (LT, D)).T

        def dwmod_cols(lo, hi):
            for j in range(lo * D // LT, hi * D // LT):
                dwm_st[:, j * LT:(j + 1) * LT] = (sc_col * dmod_s[:, j * LT:(j + 1) * LT]).astype(BF16)

        def p_in(idx):
            return pltpu.make_async_copy(p_hbm.at[idx], hb.at[idx % 4], sem_p.at[idx % 4])

        def keys(ref, lo, n):
            return _up(ref[_pr(lo, n), :])[:, 0:AR]

        def bwd_step(t_next, pn, dn, recompute, t_cur, pc, dc):
            hn = t_next // NQ
            if recompute:
                qa = QA[hn, :, _lanes(t_next)]
            doa = DOA[hn, :, _lanes(t_next)]
            if t_cur is not None:
                hc = t_cur // NQ
                qt = QA[hc, 0:DH, _lanes(t_cur)]
                dot_ = DOA[hc, 0:DH, _lanes(t_cur)]
                dq = jnp.zeros((DH, W), F32)

            def stage1(lo):
                if recompute:
                    s = _dot(keys(KA, lo, SUB_B), qa)
                dp = _dot(keys(VA, lo, SUB_B), doa)
                if recompute:
                    p = jnp.exp2(s)
                    pn[_pr(lo, SUB_B), :] = _pk(p.astype(BF16))
                else:
                    p = _up(pn[_pr(lo, SUB_B), :]).astype(F32)
                dn[_pr(lo, SUB_B), :] = _pk((p * dp).astype(BF16))

            half = KC_B // 2
            for c in range(S // KC_B):
                sl = slice(c * KC_B, (c + 1) * KC_B)
                for lo in range(c * KC_B, c * KC_B + half, SUB_B):
                    stage1(lo)
                if t_cur is not None:
                    ds = _up(dc[_pr(c * KC_B, KC_B), :])
                    dkT[:, sl] += _dot_nt(qt, ds)
                for lo in range(c * KC_B + half, (c + 1) * KC_B, SUB_B):
                    stage1(lo)
                if t_cur is not None:
                    dvT[:, sl] += _dot_nt(dot_, _up(pc[_pr(c * KC_B, KC_B), :]))
                    dq = dq + _dot(KT[:, sl], ds)
            if t_cur is not None:
                dqT[pl.ds(pl.multiple_of(hc * (DH // 2), DH // 2), DH // 2), _lanes(t_cur)] = _pk(
                    (dq * 0.25).astype(BF16))

        with _scope("P9"):
            p_in(0).start()
            p_in(1).start()
            cp_wmod.start()
            dwmod_cols(2, 6)
            cp_dwm_b.start()
            wqp[...] = _pk(wq_ref[...])
            dwq_acc[...] = jnp.zeros(dwq_acc.shape, F32)
            dkT[...] = jnp.zeros(dkT.shape, F32)
            dvT[...] = jnp.zeros(dvT.shape, F32)
            bwd_step(0, pb0, db0, True, None, None, None)

            def bwd_body(it, carry):
                t = 4 * it
                pv = pres.at[it]
                ha = hb.at[(2 * it) % 4]
                hc = hb.at[(2 * it + 1) % 4]
                p_in(2 * it).wait()
                p_in(2 * it + 1).wait()

                @pl.when(it + 1 < NIT)
                def _():
                    p_in(2 * it + 2).start()
                    p_in(2 * it + 3).start()
                bwd_step(t + 1, ha, db1, False, t, pb0, db0)
                bwd_step(t + 2, pv, db0, False, t + 1, ha, db1)
                bwd_step(t + 3, hc, db1, False, t + 2, pv, db0)
                bwd_step(jnp.minimum(t + 4, NT - 1), pb0, db0, True, t + 3, hc, db1)
                return carry
            lax.fori_loop(0, NIT, bwd_body, 0)

        def p10_mm(i, hbuf):
            tl = _tile(i, LT)
            dqc = _up(dqT[:, tl])
            kvc = dkv_s[:, tl]
            for m in range(0, D, 256):
                hbuf[m:m + 256, :] = _dot(_up(wqp[_pr(m, 256), :]), dqc) + _dot(wkv_n[m:m + 256], kvc)
            for m in range(0, D, 256):
                dwq_acc[m:m + 256, :] += _dot_nt(_up(h1T[_pr(m, 256), tl]), dqc)

        def p10_ew(i, hbuf):
            tl = _tile(i, LT)
            mu, r = st[0:1, tl], st[1:2, tl]
            for rs in _blocks(D, LT):
                nb[rs, :] = (x_raw[tl, rs].T.astype(F32) - mu) * r
            s1 = s2 = z8
            for rs in _blocks(D, RB):
                dh1 = hbuf[rs, :]
                n1 = nb[rs, :]
                acc_s[1, rs] += dh1 * n1
                acc_s[0, rs] += dh1
                dn1 = dh1 * modc[1, rs]
                hbuf[rs, :] = dn1
                s1 = s1 + _bsum(dn1)
                s2 = s2 + _bsum(dn1 * n1)
            m1 = _fin(s1) * inv_d
            m2 = _fin(s2) * inv_d
            for rs in _blocks(D, LT):
                dx0 = dxT[rs, tl] + r * (hbuf[rs, :] - m1 - nb[rs, :] * m2)
                x_raw[tl, rs] = dx0.astype(BF16).T
            cp_dx(i).start()

        with _scope("P10"):
            dkv = jnp.concatenate([dkT[...] * LN2, dvT[...]], axis=0).astype(BF16)
            dkv_s[...] = dkv
            wkv_n = wkvT.T
            pipeline(NLT, p10_mm, p10_ew, (ta, tb))
            dwkvT = _dot_nt(dkv_s[...], _up(h1T[...]))
            dwk_ref[...] = dwkvT[0:DH].astype(BF16)
            dwv_ref[...] = dwkvT[DH:2 * DH].astype(BF16)
            dwq_ref[...] = dwq_acc[...].astype(BF16)

        with _scope("P11"):
            for r in (0, 1):
                dmod_s[:, r * D:(r + 1) * D] = _row_of(acc_s[r])
            dwmod_cols(0, 2)
            cp_dwm_a.start()
            cp_wmod.wait()
            dsc = _dot_nt(jnp.broadcast_to(dmod_s[...], (16, 6 * D)).astype(BF16), wmod_v[...])[0:1]
            dc_ref[...] = (dsc * (csig * (1.0 + cvec * (1.0 - csig)))).astype(BF16)
            for i in range(NLT):
                cp_out(i).wait()
                cp_dw2(i).wait()
                cp_dw1(i).wait()
                cp_dx(i).wait()
            cp_dwm_b.wait()
            cp_dwm_a.wait()

    pl.run_scoped(scope3, V((S // 2, W), U32), V((4, S // 2, W), U32), V((S // 2, W), U32), V((S // 2, W), U32),
                  V((D // 2, S), U32), V((DH, S), F32), V((DH, S), F32), V((2 * DH, S), BF16),
                  V((D, 6 * D), BF16), V((D, 6 * D), BF16), V((D, D), F32), V((D // 2, D), U32),
                  V((D, LT), F32), V((D, LT), F32), V((D, LT), F32))


@jax.jit
def pallas_adaLN_cond__grouped_kv_mqa__mixer_token_mlp__prompt_kernel(
    A_x: jax.Array,
    A_wq: jax.Array,
    A_wk: jax.Array,
    A_wv: jax.Array,
    A_wo: jax.Array,
    B_x: jax.Array,
    B_w1: jax.Array,
    B_b1: jax.Array,
    B_w2: jax.Array,
    B_b2: jax.Array,
    c: jax.Array,
    w_mod: jax.Array,
    grad_out: jax.Array,
):
    del B_x
    any_spec = pl.BlockSpec(memory_space=pl.ANY)
    vmem_spec = pl.BlockSpec(memory_space=pltpu.VMEM)
    sds = jax.ShapeDtypeStruct
    out_shape = (
        sds((S, D), BF16), sds((S, D), BF16),
        sds((D, D), BF16), sds((DH, D), BF16), sds((DH, D), BF16), sds((D, D), BF16),
        sds((F, S), BF16), sds((1, F), BF16), sds((F, S), BF16), sds((1, S), BF16),
        sds((1, D), BF16), sds((D, 6 * D), BF16),
        sds((2 * NIT, S // 2, W), U32),
    )
    in_specs = [any_spec, vmem_spec, vmem_spec, vmem_spec, vmem_spec, any_spec, vmem_spec, any_spec,
                vmem_spec, vmem_spec, any_spec, any_spec]
    out_specs = (any_spec, any_spec, vmem_spec, vmem_spec, vmem_spec, vmem_spec, any_spec, vmem_spec,
                 any_spec, vmem_spec, vmem_spec, any_spec, any_spec)
    V = pltpu.VMEM
    scratch = [
        V((NIT, S // 2, W), U32),
        V((H, AR, S), BF16), V((H, AR, S), BF16),
        V((S // 2, LT), U32), V((S // 2, LT), U32), V((DH, S), BF16), V((DH, S), BF16),
        V((S, D), BF16), V((S, D), BF16), V((F, S), BF16), V((F, S), BF16),
        V((D // 2, S), U32), V((D // 2, S), U32), V((D // 2, S), U32),
        V((D, S), F32), V((8, S), F32),
        V((6, D, LT), F32), V((1, 6 * D), F32), V((6, D, LT), F32),
        V((D // 2, D), U32), V((D // 2, D), U32), V((1, F), F32), V((1, S), F32), V((1, 6 * D), F32),
        pltpu.SemaphoreType.DMA((6,)), pltpu.SemaphoreType.DMA((6,)), pltpu.SemaphoreType.DMA((4,)),
    ]
    res = pl.pallas_call(
        _kernel,
        out_shape=out_shape,
        in_specs=in_specs,
        out_specs=out_specs,
        scratch_shapes=scratch,
        compiler_params=pltpu.CompilerParams(vmem_limit_bytes=127 * 1024 * 1024),
    )(A_x.reshape(S, D), A_wq, A_wk.T, A_wv.T, A_wo, B_w1.T, B_b1, B_w2, B_b2,
      c, w_mod, grad_out.reshape(S, D))
    (out, dx, dwq, dwk, dwv, dwo, dw1, db1, dw2, db2, dc, dwmod, _) = res
    return (out.reshape(1, S, D), dx.reshape(1, S, D), dwq, dwk.T, dwv.T, dwo, dw1.T, db1.reshape(F), dw2,
            db2.reshape(S), dc, dwmod)
```

```python
import contextlib
import functools

import jax
import jax.numpy as jnp
from jax import lax
import jax.experimental.pallas as pl
import jax.experimental.pallas.tpu as pltpu

S, D, H, DH, F = 2048, 512, 32, 16, 1376
EPS = 1e-5
LOG2E = 1.4426950408889634
LN2 = 0.6931471805599453
QSCALE = 0.25 * LOG2E
C0 = 0.7978845608028654
C1 = 0.044715

LT = 128
NLT = S // LT
W = 256
NQ = S // W
NT = H * NQ
NIT = NT // 4
NV2 = 10
KC_F = 512
SUB_F = 256
KC_B = 256
SUB_B = 64
MB = 256
RB = 64
AR = 32
NFC = F // 128
FT = F % 128
SAFE_BOUND = 40.0

_PROFILE = False


def _scope(name):
    return jax.named_scope(name) if _PROFILE else contextlib.nullcontext()


F32 = jnp.float32
BF16 = jnp.bfloat16
U32 = jnp.uint32
NT_DIMS = (((1,), (1,)), ((), ()))


def _dot(a, b):
    return jnp.dot(a, b, preferred_element_type=F32)


def _dot_nt(a, b):
    return lax.dot_general(a, b, NT_DIMS, preferred_element_type=F32)


def _tile(i, n):
    return pl.ds(pl.multiple_of(i * n, n), n)


def _pk(x):
    return pltpu.bitcast(x, U32)


def _up(x):
    return pltpu.bitcast(x, BF16)


def _pr(m, n):
    return slice(m // 2, (m + n) // 2)


def _split3(x):
    hi = x.astype(BF16).astype(F32)
    r = x - hi
    mid = r.astype(BF16).astype(F32)
    lo = (r - mid).astype(BF16).astype(F32)
    return hi, mid, lo


def _rows16(vals, shape, axis):
    row = lax.broadcasted_iota(jnp.int32, shape, axis)
    blk = jnp.zeros(shape, F32)
    for k, v in enumerate(vals):
        blk = jnp.where(row == k, v, blk)
    return blk.astype(BF16)


def _bsum(x):
    return x.reshape(x.shape[0] // 8, 8, x.shape[1]).sum(axis=0)


def _fin(s8):
    return jnp.sum(s8, axis=0, keepdims=True)


def _moments(s1, s2, c):
    d = _fin(s1) * (1.0 / D)
    var = jnp.maximum(_fin(s2) * (1.0 / D) - d * d, 0.0)
    return c + d, lax.rsqrt(var + EPS)


def _row_of(acc):
    return jnp.sum(acc.T, axis=0, keepdims=True)


def _lanes(t):
    return pl.ds(pl.multiple_of((t % NQ) * W, W), W)


def _slot0(it):
    return jnp.where(it < NIT, jnp.clip(it - (NIT - NV2 - 1), 0, NV2), 0)


def _blocks(n, step):
    return [slice(m, min(m + step, n)) for m in range(0, n, step)]


def _kernel(
    x_hbm, wq_hbm, wk_ref, wv_ref, wo_hbm, w1_hbm, b1_ref, w2_hbm, b2_ref, c_ref, wmod_hbm, go_hbm,
    out_hbm, dx_hbm, dwq_hbm, dwk_ref, dwv_ref, dwo_hbm, dw1_hbm, db1_ref, dw2_hbm, db2_ref, dc_ref, dwmod_hbm,
    p_hbm,
    pres, pres2, QA, KA, VA, KT, VT, x_raw, go_raw, w1_v, w2_v, oT, h1T, goT, dx1b, st, modc, modrow, acc_s,
    wq_ref, wo_ref, woT_s, wqT_s, b1v, b2v, db1v, db2v, dmod_s,
    sem_in, sem_out, sem_p,
):
    V = pltpu.VMEM
    cp_xa = pltpu.make_async_copy(x_hbm.at[0:S // 2], x_raw.at[0:S // 2], sem_in.at[0])
    cp_xb = pltpu.make_async_copy(x_hbm.at[S // 2:S], x_raw.at[S // 2:S], sem_in.at[8])
    cp_w1 = pltpu.make_async_copy(w1_hbm, w1_v, sem_in.at[2])
    cp_w2 = pltpu.make_async_copy(w2_hbm, w2_v, sem_in.at[3])
    cp_go = pltpu.make_async_copy(go_hbm, go_raw, sem_in.at[4])
    cp_wq = pltpu.make_async_copy(wq_hbm, wq_ref, sem_in.at[6])
    cp_wo = pltpu.make_async_copy(wo_hbm, wo_ref, sem_in.at[7])
    cp_dwq = pltpu.make_async_copy(wq_ref, dwq_hbm, sem_out.at[6])
    cp_dwo = pltpu.make_async_copy(wo_ref, dwo_hbm, sem_out.at[7])

    def cp_out(i):
        return pltpu.make_async_copy(go_raw.at[_tile(i, LT), :], out_hbm.at[_tile(i, LT), :], sem_out.at[0])

    def cp_dw2(i):
        return pltpu.make_async_copy(w2_v.at[:, _tile(i, LT)], dw2_hbm.at[:, _tile(i, LT)], sem_out.at[1])

    def cp_dw1(i):
        return pltpu.make_async_copy(w1_v.at[:, _tile(i, LT)], dw1_hbm.at[:, _tile(i, LT)], sem_out.at[2])

    def cp_dx(i):
        return pltpu.make_async_copy(x_raw.at[_tile(i, LT), :], dx_hbm.at[_tile(i, LT), :], sem_out.at[3])

    cvec = c_ref[...].astype(F32)
    csig = jax.nn.sigmoid(cvec)
    sc = cvec * csig
    wkvT = jnp.concatenate([wk_ref[...], wv_ref[...]], axis=0)
    z8 = jnp.zeros((8, LT), F32)
    inv_d = 1.0 / D

    def pipeline(n, mm, ew, bufs, lo=0):
        mm(lo, bufs[0])

        def body(j, carry):
            i = lo + 2 * j
            ew(i, bufs[0])
            mm(i + 1, bufs[1])
            ew(i + 1, bufs[1])
            mm(i + 2, bufs[0])
            return carry
        lax.fori_loop(0, (n - lo) // 2 - 1, body, 0)
        ew(n - 2, bufs[0])
        mm(n - 1, bufs[1])
        ew(n - 1, bufs[1])

    def scope1(wmod_v, kv_s, xb, h1a, h1b, qn_s, hb, l0, l1):
        def mod_parts(lo, hi):
            mod = _dot(jnp.broadcast_to(sc, (16, D)).astype(BF16), wmod_v[:, lo * D:hi * D])[0:1]
            modrow[:, lo * D:hi * D] = mod
            for r in range(lo, hi):
                m_r = mod[:, (r - lo) * D:(r - lo + 1) * D]
                if r in (1, 4):
                    m_r = m_r + 1.0
                modc[r] = jnp.broadcast_to(m_r, (LT, D)).T

        with _scope("P1"):
            cp_wma = pltpu.make_async_copy(wmod_hbm.at[:, 0:2 * D], wmod_v.at[:, 0:2 * D], sem_in.at[1])
            cp_wmb = pltpu.make_async_copy(wmod_hbm.at[:, 2 * D:6 * D], wmod_v.at[:, 2 * D:6 * D], sem_in.at[5])
            cp_wma.start()
            cp_xa.start()
            cp_wq.start()
            cp_xb.start()
            b1v[...] = b1_ref[...].astype(F32).reshape(1, F)
            b2v[...] = b2_ref[...].astype(F32).reshape(1, S)
            qn_s[...] = jnp.zeros(qn_s.shape, F32)
            cp_wma.wait()
            mod_parts(0, 2)
            cp_wq.wait()
            wqT_s[...] = _pk(wq_ref[...].T)

        with _scope("P2"):
            cp_xa.wait()
            cp_wmb.start()
            cp_wo.start()
            cp_go.start()
            cp_w2.start()

            def ln1_chunk(i, hbuf):
                tl = _tile(i, LT)
                for rs in _blocks(D, LT):
                    xb[rs, :] = x_raw[tl, rs].T.astype(F32)
                c = xb[0:1, :]
                s1 = s2 = z8
                for rs in _blocks(D, RB):
                    d = xb[rs, :] - c
                    s1 = s1 + _bsum(d)
                    s2 = s2 + _bsum(d * d)
                mu, r = _moments(s1, s2, c)
                st[0:1, tl] = mu
                st[1:2, tl] = r
                for rs in _blocks(D, RB):
                    h1 = _pk((((xb[rs, :] - mu) * r) * modc[1, rs] + modc[0, rs]).astype(BF16))
                    hbuf[_pr(rs.start, RB), :] = h1
                    h1T[_pr(rs.start, RB), tl] = h1

            def proj_chunk(i, hbuf):
                tl = _tile(i, LT)
                h1 = _up(hbuf[...])
                kv_s[:, tl] = _dot(wkvT, h1)
                for m in range(0, D, 256):
                    q = (_dot(_up(wqT_s[_pr(m, 256), :]), h1) * QSCALE).astype(BF16)
                    q3 = q.reshape(256 // DH, DH, LT)
                    hs = slice(m // DH, (m + 256) // DH)
                    QA[hs, 0:DH, tl] = q3
                    QA[hs, DH:AR, tl] = jnp.zeros((256 // DH, AR - DH, LT), BF16)
                    qf = q3.astype(F32)
                    qn_s[...] = jnp.maximum(qn_s[...], jnp.max(jnp.sum(qf * qf, axis=1), axis=0, keepdims=True))

            pipeline(NLT // 2, ln1_chunk, proj_chunk, (h1a, h1b))
            cp_xb.wait()
            pipeline(NLT, ln1_chunk, proj_chunk, (h1a, h1b), lo=NLT // 2)

        with _scope("P3"):
            kvT = kv_s[...]
            kTb = kvT[0:DH].astype(BF16)
            vTb = kvT[DH:2 * DH].astype(BF16)
            KT[...] = kTb
            VT[...] = vTb
            rows = lax.broadcasted_iota(jnp.int32, (LT - DH, S), 0)
            tail = jnp.where(rows < 3, 1.0, 0.0).astype(BF16)
            ka_t = jnp.concatenate([kTb, tail], axis=0)
            va_t = jnp.concatenate([vTb, tail], axis=0)
            for j in range(NLT):
                KA[_pr(j * LT, LT), :] = _pk(ka_t[:, j * LT:(j + 1) * LT].T)
                VA[_pr(j * LT, LT), :] = _pk(va_t[:, j * LT:(j + 1) * LT].T)

            kf = kTb.astype(F32)
            kn2 = jnp.max(jnp.sum(kf * kf, axis=0, keepdims=True))
            bound2 = jnp.max(qn_s[...]) * kn2
            vmax = jnp.max(jnp.abs(vTb.astype(F32)))
            safe = jnp.logical_and(bound2 <= SAFE_BOUND * SAFE_BOUND, vmax <= 1e15)

            cp_wmb.wait()
            mod_parts(2, 6)
            cp_wo.wait()
            woT_s[...] = _pk(wo_ref[...].T)
            cp_go.wait()

        def keys(ref, lo, n):
            return _up(ref[_pr(lo, n), :])[:, 0:AR]

        with _scope("P4max"):
            @pl.when(jnp.logical_not(safe))
            def _():
                def pmax(t, carry):
                    h = t // NQ
                    q = QA[h, :, _lanes(t)]
                    m = None
                    for lo in range(0, S, KC_F):
                        mc = jnp.max(_dot(keys(KA, lo, KC_F), q), axis=0, keepdims=True)
                        m = mc if m is None else jnp.maximum(m, mc)
                    hi, mid, lo_ = _split3(m)
                    QA[h, DH:AR, _lanes(t)] = _rows16((-hi, -mid, -lo_), (AR - DH, W), 0)
                    return carry
                lax.fori_loop(0, NT, pmax, 0)

        def p_out(idx):
            return pltpu.make_async_copy(hb.at[idx % 4], p_hbm.at[idx], sem_p.at[idx % 4])

        def fwd_step(t_next, pn, ln, t_cur, pc, lc):
            q = QA[t_next // NQ, :, _lanes(t_next)]
            lacc = jnp.zeros((32, W), F32)
            o = jnp.zeros((DH, W), F32)
            for c in range(S // KC_F):
                for lo in range(c * KC_F, (c + 1) * KC_F, SUB_F):
                    p = jnp.exp2(_dot(keys(KA, lo, SUB_F), q))
                    pn[_pr(lo, SUB_F), :] = _pk(p.astype(BF16))
                    lacc = lacc + p.reshape(SUB_F // 32, 32, W).sum(axis=0)
                if t_cur is not None:
                    for lo in range(c * KC_F, (c + 1) * KC_F, 128):
                        o = o + _dot(VT[:, lo:lo + 128], _up(pc[_pr(lo, 128), :]))
            lnew = lacc.sum(axis=0, keepdims=True)
            if t_cur is not None:
                hc = t_cur // NQ
                linv = 1.0 / lc[...]
                oT[pl.ds(pl.multiple_of(hc * (DH // 2), DH // 2), DH // 2), _lanes(t_cur)] = _pk(
                    (o * linv).astype(BF16))
                sh = QA[hc, DH:AR, _lanes(t_cur)].astype(F32)
                hi, mid, lo = _split3(linv)
                QA[hc, DH:AR, _lanes(t_cur)] = _rows16(
                    (sh[0:1], sh[1:2], sh[2:3], hi, mid, lo), (AR - DH, W), 0)
            ln[...] = lnew

        with _scope("P4"):
            fwd_step(0, pres2.at[0], l0, None, None, None)

            def fwd_body(it, carry):
                t = 4 * it
                pv = pres.at[it]
                ha = hb.at[(2 * it) % 4]
                hc = hb.at[(2 * it + 1) % 4]
                p0 = pres2.at[_slot0(it)]
                p0n = pres2.at[_slot0(it + 1)]

                @pl.when(it >= 2)
                def _():
                    p_out(2 * it - 4).wait()
                    p_out(2 * it - 3).wait()
                goT[_tile(it % 4, LT // 2), _tile(it // 4, LT)] = _pk(
                    go_raw[_tile(it // 4, LT), _tile(it % 4, LT)].T)
                fwd_step(t + 1, ha, l1, t, p0, l0)
                p_out(2 * it).start()
                fwd_step(t + 2, pv, l0, t + 1, ha, l1)
                fwd_step(t + 3, hc, l1, t + 2, pv, l0)
                p_out(2 * it + 1).start()
                fwd_step(jnp.minimum(t + 4, NT - 1), p0n, l0, t + 3, hc, l1)
                return carry
            lax.fori_loop(0, NIT, fwd_body, 0)
            cp_w1.start()
            for k in range(4):
                p_out(2 * NIT - 4 + k).wait()

    pl.run_scoped(scope1, V((D, 6 * D), BF16), V((2 * DH, S), F32), V((D, LT), F32),
                  V((D // 2, LT), U32), V((D // 2, LT), U32), V((1, LT), F32),
                  V((4, S // 2, W), U32),
                  V((1, W), F32), V((1, W), F32))

    def scope2(x1T, h3T, g_s, gT_s, du_s, duT_s, dgbuf, ta, tb, tc, td):
        def a_mm(i, abuf):
            och = _up(oT[:, _tile(i, LT)])
            for m in range(0, D, 256):
                abuf[m:m + 256, :] = _dot(_up(woT_s[_pr(m, 256), :]), och)

        def dg_mm(sl):
            w2r = w2_v[sl, :]
            for m in range(0, D, 256):
                dgbuf[m:m + 256, sl] = _dot_nt(_up(goT[_pr(m, 256), :]), w2r)

        def p5_ew(i, abuf):
            tl = _tile(i, LT)
            for rs in _blocks(D, LT):
                x1T[rs, tl] = x_raw[tl, rs].T.astype(F32) + modc[2, rs] * abuf[rs, :]
            c = x1T[0:1, tl]
            s1 = s2 = z8
            for rs in _blocks(D, RB):
                d = x1T[rs, tl] - c
                s1 = s1 + _bsum(d)
                s2 = s2 + _bsum(d * d)
            mu2, r2 = _moments(s1, s2, c)

            def h2_of(rs):
                return ((x1T[rs, tl] - mu2) * r2) * modc[4, rs] + modc[3, rs]
            c3 = h2_of(slice(0, 8))[0:1]
            s1 = s2 = z8
            for rs in _blocks(D, RB):
                d = h2_of(rs) - c3
                s1 = s1 + _bsum(d)
                s2 = s2 + _bsum(d * d)
            mu3, r3 = _moments(s1, s2, c3)
            st[2:3, tl] = mu2
            st[3:4, tl] = r2
            st[4:5, tl] = mu3
            st[5:6, tl] = r3
            for rs in _blocks(D, RB):
                h3T[_pr(rs.start, RB), tl] = _pk(((h2_of(rs) - mu3) * r3).astype(BF16))

        with _scope("P5"):
            a_mm(0, ta)

            def p5a(j, carry):
                i = 2 * j
                p5_ew(i, ta)
                a_mm(i + 1, tb)
                p5_ew(i + 1, tb)
                a_mm(i + 2, ta)
                return carry
            lax.fori_loop(0, 2, p5a, 0)
            p5_ew(4, ta)
            a_mm(5, tb)
            cp_w2.wait()
            p5_ew(5, tb)
            a_mm(6, ta)
            dg_mm(slice(NFC * 128, F))

            def p5b(j, carry):
                i = 6 + 2 * j
                p5_ew(i, ta)
                a_mm(i + 1, tb)
                dg_mm(_tile(2 * j, 128))
                p5_ew(i + 1, tb)
                a_mm(jnp.minimum(i + 2, NLT - 1), ta)
                dg_mm(_tile(2 * j + 1, 128))
                return carry
            lax.fori_loop(0, NFC // 2, p5b, 0)

        def u_mm(sl, n, ubuf):
            w1r = w1_v[sl, :]
            for m in range(0, D, 256):
                ubuf[m:m + 256, 0:n] = _dot_nt(_up(h3T[_pr(m, 256), :]), w1r)

        def f_ew(sl, sl2, n, ubuf):
            b1r = b1v[:, sl]
            sdb = jnp.zeros((8, n), F32)
            for rs in _blocks(D, LT):
                gb = modc[5, rs, 0:n]
                u = ubuf[rs, 0:n] + b1r
                u2 = u * u
                t = jnp.tanh(C0 * u * (1.0 + C1 * u2))
                hp = 0.5 * (1.0 + t)
                g = u * hp
                du = (dgbuf[rs, sl] * gb) * (hp + 0.5 * u * (1.0 - t * t) * C0 * (1.0 + 3.0 * C1 * u2))
                dub = du.astype(BF16)
                g_s[_pr(rs.start, LT), sl] = _pk(g.astype(BF16))
                du_s[_pr(rs.start, LT), sl] = _pk(dub)
                gT_s[sl2, rs] = _pk((g * gb).astype(BF16).T)
                duT_s[sl2, rs] = _pk(dub.T)
                sdb = sdb + _bsum(du)
            db1v[:, sl] = _fin(sdb)

        with _scope("P6"):
            cp_w1.wait()
            u_mm(slice(0, 128), 128, ta)

            def p6(j, carry):
                i = 2 * j
                f_ew(_tile(i, 128), _tile(i, 64), 128, ta)
                u_mm(_tile(i + 1, 128), 128, tb)
                f_ew(_tile(i + 1, 128), _tile(i + 1, 64), 128, tb)
                u_mm(_tile(i + 2, 128), 128, ta)
                return carry
            lax.fori_loop(0, NFC // 2 - 1, p6, 0)
            i8, i9 = NFC - 2, NFC - 1
            f_ew(slice(i8 * 128, i9 * 128), slice(i8 * 64, i9 * 64), 128, ta)
            u_mm(slice(i9 * 128, NFC * 128), 128, tb)
            f_ew(slice(i9 * 128, NFC * 128), slice(i9 * 64, NFC * 64), 128, tb)
            u_mm(slice(NFC * 128, F), FT, ta)
            f_ew(slice(NFC * 128, F), slice(NFC * 64, F // 2), FT, ta)

        def p7_mm(i, bufs):
            yb, hb_ = bufs
            tl = _tile(i, LT)
            w2c = w2_v[:, tl]
            w1c = w1_v[:, tl]
            for m in range(0, D, MB):
                yb[m:m + MB, :] = _dot(_up(g_s[_pr(m, MB), :]), w2c)
            for m in range(0, D, MB):
                hb_[m:m + MB, :] = _dot(_up(du_s[_pr(m, MB), :]), w1c)
            goc = _up(goT[:, tl])
            h3c = _up(h3T[:, tl])
            for rs in _blocks(F, MB):
                w2_v[rs, tl] = _dot(_up(gT_s[_pr(rs.start, rs.stop - rs.start), :]), goc).astype(BF16)
            for rs in _blocks(F, MB):
                w1_v[rs, tl] = _dot(_up(duT_s[_pr(rs.start, rs.stop - rs.start), :]), h3c).astype(BF16)
            cp_dw2(i).start()
            cp_dw1(i).start()

        def p7_ew(i, bufs):
            yb, hb_ = bufs
            tl = _tile(i, LT)
            b2r = b2v[:, tl]
            mu2, r2, mu3, r3 = st[2:3, tl], st[3:4, tl], st[4:5, tl], st[5:6, tl]
            for rs in _blocks(D, LT):
                go_raw[tl, rs] = (x1T[rs, tl] + modc[5, rs] * (yb[rs, :] + b2r)).astype(BF16).T
            cp_out(i).start()

            def norms(rs):
                n2 = (x1T[rs, tl] - mu2) * r2
                h3 = (n2 * modc[4, rs] + modc[3, rs] - mu3) * r3
                return n2, h3

            def dx2_of(rs):
                return _up(goT[_pr(rs.start, RB), tl]).astype(F32)

            s1 = s2 = sdb = z8
            for rs in _blocks(D, RB):
                dx2 = dx2_of(rs)
                acc_s[5, rs] += dx2 * (yb[rs, :] + b2r)
                sdb = sdb + _bsum(modc[5, rs] * dx2)
                _, h3 = norms(rs)
                dh3 = hb_[rs, :]
                s1 = s1 + _bsum(dh3)
                s2 = s2 + _bsum(dh3 * h3)
            db2v[:, tl] = _fin(sdb)
            m1 = _fin(s1) * inv_d
            m2 = _fin(s2) * inv_d
            s3 = s4 = z8
            for rs in _blocks(D, RB):
                n2, h3 = norms(rs)
                dh2 = r3 * (hb_[rs, :] - m1 - h3 * m2)
                acc_s[4, rs] += dh2 * n2
                acc_s[3, rs] += dh2
                dn2 = dh2 * modc[4, rs]
                hb_[rs, :] = dn2
                s3 = s3 + _bsum(dn2)
                s4 = s4 + _bsum(dn2 * n2)
            m3 = _fin(s3) * inv_d
            m4 = _fin(s4) * inv_d
            for rs in _blocks(D, RB):
                n2 = (x1T[rs, tl] - mu2) * r2
                dx1 = dx2_of(rs) + r2 * (hb_[rs, :] - m3 - n2 * m4)
                dx1b[_pr(rs.start, RB), tl] = _pk(dx1.astype(BF16))

        with _scope("P7"):
            acc_s[...] = jnp.zeros(acc_s.shape, F32)
            pipeline(NLT, p7_mm, p7_ew, ((ta, tb), (tc, td)))

        db1_ref[...] = db1v[...].reshape(F).astype(BF16)
        db2_ref[...] = db2v[...].reshape(S).astype(BF16)
        for r in (3, 4, 5):
            dmod_s[:, r * D:(r + 1) * D] = _row_of(acc_s[r])

    pl.run_scoped(scope2, V((D, S), F32), V((D // 2, S), U32), V((D // 2, F), U32),
                  V((F // 2, D), U32), V((D // 2, F), U32), V((F // 2, D), U32),
                  V((D, F), F32),
                  V((D, LT), F32), V((D, LT), F32), V((D, LT), F32), V((D, LT), F32))

    def scope3(DOA, dqT, dkT, dvT, wm, dsc_s):
        cp_wm = pltpu.make_async_copy(wmod_hbm, wm, sem_in.at[1])
        cp_dwm_b = pltpu.make_async_copy(wm.at[:, 2 * D:6 * D], dwmod_hbm.at[:, 2 * D:6 * D], sem_out.at[4])
        cp_dwm_a = pltpu.make_async_copy(wm.at[:, 0:2 * D], dwmod_hbm.at[:, 0:2 * D], sem_out.at[5])
        sc_col = jnp.broadcast_to(sc, (LT, D)).T

        def mod_bwd(lo, hi):
            dm = dmod_s[:, lo * D:hi * D]
            part = _dot_nt(jnp.broadcast_to(dm, (16, (hi - lo) * D)).astype(BF16), wm[:, lo * D:hi * D])[0:1]
            for j in range(lo * D // LT, hi * D // LT):
                wm[:, j * LT:(j + 1) * LT] = (sc_col * dmod_s[:, j * LT:(j + 1) * LT]).astype(BF16)
            return part

        def scope_p8(wog, m_acc, ta, tb):
            def p8_mm(i, dbuf_):
                tl = _tile(i, LT)
                dxc = _up(dx1b[:, tl])
                for m in range(0, D, 256):
                    dbuf_[m:m + 256, :] = _dot(_up(wog[_pr(m, 256), :]), dxc)
                for m in range(0, D, 256):
                    m_acc[m:m + 256, :] += _dot_nt(_up(oT[_pr(m, 256), tl]), dxc)

            def p8_ew(i, dbuf_):
                tl = _tile(i, LT)
                hpb = RB // DH
                for rs in _blocks(D, RB):
                    hs = slice(rs.start // DH, rs.stop // DH)
                    li = QA[hs, DH:AR, tl].astype(F32)
                    linv = li[:, 3:4] + li[:, 4:5] + li[:, 5:6]
                    dos = (dbuf_[rs, :].reshape(hpb, DH, LT) * linv).astype(BF16)
                    of = _up(oT[_pr(rs.start, RB), tl]).astype(F32).reshape(hpb, DH, LT)
                    delta = jnp.sum(dos.astype(F32) * of, axis=1, keepdims=True)
                    hi, mid, lo = _split3(delta)
                    DOA[hs, 0:DH, tl] = dos
                    DOA[hs, DH:AR, tl] = _rows16((-hi, -mid, -lo), (hpb, AR - DH, LT), 1)

            garow = modrow[:, 2 * D:3 * D]
            wof = wo_ref[...].astype(F32)
            wog[...] = _pk((wof * garow).astype(BF16))
            m_acc[...] = jnp.zeros(m_acc.shape, F32)
            pipeline(NLT, p8_mm, p8_ew, (ta, tb))
            m_od = m_acc[...]
            dmod_s[:, 2 * D:3 * D] = jnp.sum(m_od * wo_ref[...].astype(F32), axis=0, keepdims=True)
            wo_ref[...] = (m_od * garow).astype(BF16)
            cp_dwo.start()
            cp_wm.wait()
            dsc_s[...] = mod_bwd(2, 6)
            cp_dwm_b.start()

        with _scope("P8"):
            cp_wm.start()
            pl.run_scoped(scope_p8, V((D // 2, D), U32), V((D, D), F32), V((D, LT), F32), V((D, LT), F32))

        def scope_p9(hb, db0, db1):
            def p_in(idx):
                return pltpu.make_async_copy(p_hbm.at[idx], hb.at[idx % 4], sem_p.at[idx % 4])

            def keys(ref, lo, n):
                return _up(ref[_pr(lo, n), :])[:, 0:AR]

            def bwd_step(t_next, pn, dn, recompute, t_cur, pc, dc):
                hn = t_next // NQ
                if recompute:
                    qa = QA[hn, :, _lanes(t_next)]
                doa = DOA[hn, :, _lanes(t_next)]
                if t_cur is not None:
                    hc = t_cur // NQ
                    qt = QA[hc, 0:DH, _lanes(t_cur)]
                    dot_ = DOA[hc, 0:DH, _lanes(t_cur)]
                    dq = jnp.zeros((DH, W), F32)

                def stage1(lo):
                    if recompute:
                        s = _dot(keys(KA, lo, SUB_B), qa)
                    dp = _dot(keys(VA, lo, SUB_B), doa)
                    if recompute:
                        p = jnp.exp2(s)
                        pn[_pr(lo, SUB_B), :] = _pk(p.astype(BF16))
                    else:
                        p = _up(pn[_pr(lo, SUB_B), :]).astype(F32)
                    dn[_pr(lo, SUB_B), :] = _pk((p * dp).astype(BF16))

                half = KC_B // 2
                for c in range(S // KC_B):
                    sl = slice(c * KC_B, (c + 1) * KC_B)
                    for lo in range(c * KC_B, c * KC_B + half, SUB_B):
                        stage1(lo)
                    if t_cur is not None:
                        ds = _up(dc[_pr(c * KC_B, KC_B), :])
                        dkT[:, sl] += _dot_nt(qt, ds)
                    for lo in range(c * KC_B + half, (c + 1) * KC_B, SUB_B):
                        stage1(lo)
                    if t_cur is not None:
                        dvT[:, sl] += _dot_nt(dot_, _up(pc[_pr(c * KC_B, KC_B), :]))
                        dq = dq + _dot(KT[:, sl], ds)
                if t_cur is not None:
                    dqT[pl.ds(pl.multiple_of(hc * (DH // 2), DH // 2), DH // 2), _lanes(t_cur)] = _pk(
                        (dq * 0.25).astype(BF16))

            p_in(0).start()
            p_in(1).start()
            dkT[...] = jnp.zeros(dkT.shape, F32)
            dvT[...] = jnp.zeros(dvT.shape, F32)
            bwd_step(0, pres2.at[0], db0, True, None, None, None)

            def bwd_body(recompute, it, carry):
                t = 4 * it
                pv = pres.at[it]
                ha = hb.at[(2 * it) % 4]
                hc = hb.at[(2 * it + 1) % 4]
                p0 = pres2.at[_slot0(it)]
                p0n = pres2.at[_slot0(it + 1)]
                p_in(2 * it).wait()
                p_in(2 * it + 1).wait()

                @pl.when(it + 1 < NIT)
                def _():
                    p_in(2 * it + 2).start()
                    p_in(2 * it + 3).start()
                bwd_step(t + 1, ha, db1, False, t, p0, db0)
                bwd_step(t + 2, pv, db0, False, t + 1, ha, db1)
                bwd_step(t + 3, hc, db1, False, t + 2, pv, db0)
                bwd_step(jnp.minimum(t + 4, NT - 1), p0n, db0, recompute, t + 3, hc, db1)
                return carry
            lax.fori_loop(0, NIT - NV2 - 1, functools.partial(bwd_body, True), 0)
            lax.fori_loop(NIT - NV2 - 1, NIT, functools.partial(bwd_body, False), 0)

        with _scope("P9"):
            pl.run_scoped(scope_p9, V((4, S // 2, W), U32), V((S // 2, W), U32), V((S // 2, W), U32))

        def scope_p10(dkv_s, dwq_acc, wqp, ta, tb, nb):
            def p10_mm(i, hbuf):
                tl = _tile(i, LT)
                dqc = _up(dqT[:, tl])
                kvc = dkv_s[:, tl]
                for m in range(0, D, 256):
                    hbuf[m:m + 256, :] = _dot(_up(wqp[_pr(m, 256), :]), dqc) + _dot(wkv_n[m:m + 256], kvc)
                for m in range(0, D, 256):
                    dwq_acc[m:m + 256, :] += _dot_nt(_up(h1T[_pr(m, 256), tl]), dqc)

            def p10_ew(i, hbuf):
                tl = _tile(i, LT)
                mu, r = st[0:1, tl], st[1:2, tl]
                for rs in _blocks(D, LT):
                    nb[rs, :] = (x_raw[tl, rs].T.astype(F32) - mu) * r
                s1 = s2 = z8
                for rs in _blocks(D, RB):
                    dh1 = hbuf[rs, :]
                    n1 = nb[rs, :]
                    acc_s[1, rs] += dh1 * n1
                    acc_s[0, rs] += dh1
                    dn1 = dh1 * modc[1, rs]
                    hbuf[rs, :] = dn1
                    s1 = s1 + _bsum(dn1)
                    s2 = s2 + _bsum(dn1 * n1)
                m1 = _fin(s1) * inv_d
                m2 = _fin(s2) * inv_d
                for rs in _blocks(D, LT):
                    dx1 = _up(dx1b[_pr(rs.start, LT), tl]).astype(F32)
                    dx0 = dx1 + r * (hbuf[rs, :] - m1 - nb[rs, :] * m2)
                    x_raw[tl, rs] = dx0.astype(BF16).T
                cp_dx(i).start()

            dkv = jnp.concatenate([dkT[...] * LN2, dvT[...]], axis=0).astype(BF16)
            dkv_s[...] = dkv
            wkv_n = wkvT.T
            wqp[...] = _pk(wq_ref[...])
            dwq_acc[...] = jnp.zeros(dwq_acc.shape, F32)
            pipeline(NLT, p10_mm, p10_ew, (ta, tb))
            wq_ref[...] = dwq_acc[...].astype(BF16)
            cp_dwq.start()
            dwkvT = _dot_nt(dkv_s[...], _up(h1T[...]))
            dwk_ref[...] = dwkvT[0:DH].astype(BF16)
            dwv_ref[...] = dwkvT[DH:2 * DH].astype(BF16)

        with _scope("P10"):
            pl.run_scoped(scope_p10, V((2 * DH, S), BF16), V((D, D), F32), V((D // 2, D), U32),
                          V((D, LT), F32), V((D, LT), F32), V((D, LT), F32))

        with _scope("P11"):
            for r in (0, 1):
                dmod_s[:, r * D:(r + 1) * D] = _row_of(acc_s[r])
            dsc = dsc_s[...] + mod_bwd(0, 2)
            cp_dwm_a.start()
            dc_ref[...] = (dsc * (csig * (1.0 + cvec * (1.0 - csig)))).astype(BF16)
            for i in range(NLT):
                cp_out(i).wait()
                cp_dw2(i).wait()
                cp_dw1(i).wait()
                cp_dx(i).wait()
            cp_dwo.wait()
            cp_dwq.wait()
            cp_dwm_b.wait()
            cp_dwm_a.wait()

    pl.run_scoped(scope3, V((H, AR, S), BF16), V((D // 2, S), U32), V((DH, S), F32), V((DH, S), F32),
                  V((D, 6 * D), BF16), V((1, D), F32))


@jax.jit
def pallas_adaLN_cond__grouped_kv_mqa__mixer_token_mlp__prompt_kernel(
    A_x: jax.Array,
    A_wq: jax.Array,
    A_wk: jax.Array,
    A_wv: jax.Array,
    A_wo: jax.Array,
    B_x: jax.Array,
    B_w1: jax.Array,
    B_b1: jax.Array,
    B_w2: jax.Array,
    B_b2: jax.Array,
    c: jax.Array,
    w_mod: jax.Array,
    grad_out: jax.Array,
):
    del B_x
    any_spec = pl.BlockSpec(memory_space=pl.ANY)
    vmem_spec = pl.BlockSpec(memory_space=pltpu.VMEM)
    sds = jax.ShapeDtypeStruct
    out_shape = (
        sds((S, D), BF16), sds((S, D), BF16),
        sds((D, D), BF16), sds((DH, D), BF16), sds((DH, D), BF16), sds((D, D), BF16),
        sds((F, S), BF16), sds((F,), BF16), sds((F, S), BF16), sds((S,), BF16),
        sds((1, D), BF16), sds((D, 6 * D), BF16),
        sds((2 * NIT, S // 2, W), U32),
    )
    in_specs = [any_spec, any_spec, vmem_spec, vmem_spec, any_spec, any_spec, vmem_spec, any_spec,
                vmem_spec, vmem_spec, any_spec, any_spec]
    out_specs = (any_spec, any_spec, any_spec, vmem_spec, vmem_spec, any_spec, any_spec, vmem_spec,
                 any_spec, vmem_spec, vmem_spec, any_spec, any_spec)
    V = pltpu.VMEM
    scratch = [
        V((NIT, S // 2, W), U32), V((NV2 + 1, S // 2, W), U32),
        V((H, AR, S), BF16),
        V((S // 2, LT), U32), V((S // 2, LT), U32), V((DH, S), BF16), V((DH, S), BF16),
        V((S, D), BF16), V((S, D), BF16), V((F, S), BF16), V((F, S), BF16),
        V((D // 2, S), U32), V((D // 2, S), U32), V((D // 2, S), U32),
        V((D // 2, S), U32), V((8, S), F32),
        V((6, D, LT), F32), V((1, 6 * D), F32), V((6, D, LT), F32),
        V((D, D), BF16), V((D, D), BF16),
        V((D // 2, D), U32), V((D // 2, D), U32), V((1, F), F32), V((1, S), F32),
        V((1, F), F32), V((1, S), F32), V((1, 6 * D), F32),
        pltpu.SemaphoreType.DMA((9,)), pltpu.SemaphoreType.DMA((8,)), pltpu.SemaphoreType.DMA((4,)),
    ]
    res = pl.pallas_call(
        _kernel,
        out_shape=out_shape,
        in_specs=in_specs,
        out_specs=out_specs,
        scratch_shapes=scratch,
        compiler_params=pltpu.CompilerParams(vmem_limit_bytes=127 * 1024 * 1024),
    )(A_x.reshape(S, D), A_wq, A_wk.T, A_wv.T, A_wo, B_w1.T, B_b1, B_w2, B_b2,
      c, w_mod, grad_out.reshape(S, D))
    (out, dx, dwq, dwk, dwv, dwo, dw1, db1, dw2, db2, dc, dwmod, _) = res
    return (out.reshape(1, S, D), dx.reshape(1, S, D), dwq, dwk.T, dwv.T, dwo, dw1.T, db1, dw2,
            db2, dc, dwmod)
```

```python
import contextlib
import functools

import jax
import jax.numpy as jnp
from jax import lax
import jax.experimental.pallas as pl
import jax.experimental.pallas.tpu as pltpu

S, D, H, DH, F = 2048, 512, 32, 16, 1376
EPS = 1e-5
LOG2E = 1.4426950408889634
LN2 = 0.6931471805599453
QSCALE = 0.25 * LOG2E
C0 = 0.7978845608028654
C1 = 0.044715

LT = 128
NLT = S // LT
W = 256
NQ = S // W
NT = H * NQ
NIT = NT // 4
NV2 = 10
KC_F = 512
SUB_F = 256
KC_B = 256
SUB_B = 64
MB = 256
RB = 64
AR = 32
NFC = F // 128
FT = F % 128
SAFE_BOUND = 40.0

_PROFILE = False


def _scope(name):
    return jax.named_scope(name) if _PROFILE else contextlib.nullcontext()


F32 = jnp.float32
BF16 = jnp.bfloat16
U32 = jnp.uint32
NT_DIMS = (((1,), (1,)), ((), ()))


def _dot(a, b):
    return jnp.dot(a, b, preferred_element_type=F32)


def _dot_nt(a, b):
    return lax.dot_general(a, b, NT_DIMS, preferred_element_type=F32)


def _tile(i, n):
    return pl.ds(pl.multiple_of(i * n, n), n)


def _pk(x):
    return pltpu.bitcast(x, U32)


def _up(x):
    return pltpu.bitcast(x, BF16)


def _pr(m, n):
    return slice(m // 2, (m + n) // 2)


def _split3(x):
    hi = x.astype(BF16).astype(F32)
    r = x - hi
    mid = r.astype(BF16).astype(F32)
    lo = (r - mid).astype(BF16).astype(F32)
    return hi, mid, lo


def _rows16(vals, shape, axis):
    row = lax.broadcasted_iota(jnp.int32, shape, axis)
    blk = jnp.zeros(shape, F32)
    for k, v in enumerate(vals):
        blk = jnp.where(row == k, v, blk)
    return blk.astype(BF16)


def _bsum(x):
    return x.reshape(x.shape[0] // 8, 8, x.shape[1]).sum(axis=0)


def _fin(s8):
    return jnp.sum(s8, axis=0, keepdims=True)


def _moments(s1, s2, c):
    d = _fin(s1) * (1.0 / D)
    var = jnp.maximum(_fin(s2) * (1.0 / D) - d * d, 0.0)
    return c + d, lax.rsqrt(var + EPS)


def _row_of(acc):
    return jnp.sum(acc.T, axis=0, keepdims=True)


def _lanes(t):
    return pl.ds(pl.multiple_of((t % NQ) * W, W), W)


def _slot0(it):
    return jnp.maximum(it - (NIT - NV2 - 1), 0)


def _blocks(n, step):
    return [slice(m, min(m + step, n)) for m in range(0, n, step)]


def _kernel(
    x_hbm, wq_hbm, wk_ref, wv_ref, wo_hbm, w1_hbm, b1_ref, w2_hbm, b2_ref, c_ref, wmod_hbm, go_hbm,
    out_hbm, dx_hbm, dwq_hbm, dwk_ref, dwv_ref, dwo_hbm, dw1_hbm, db1_ref, dw2_hbm, db2_ref, dc_ref, dwmod_hbm,
    p_hbm,
    pres, pres2, QA, KA, VA, KT, VT, x_raw, go_raw, w1_v, w2_v, oT, h1T, goT, dx1b, st, modc, modrow, acc_s,
    wq_ref, wo_ref, woT_s, wqT_s, b1v, b2v, db1v, db2v, dmod_s,
    sem_in, sem_out, sem_p,
):
    V = pltpu.VMEM
    cp_xa = pltpu.make_async_copy(x_hbm.at[0:S // 2], x_raw.at[0:S // 2], sem_in.at[0])
    cp_xb = pltpu.make_async_copy(x_hbm.at[S // 2:S], x_raw.at[S // 2:S], sem_in.at[8])
    cp_w1 = pltpu.make_async_copy(w1_hbm, w1_v, sem_in.at[2])
    cp_w2a = pltpu.make_async_copy(w2_hbm.at[0:D], w2_v.at[0:D], sem_in.at[3])
    cp_w2b = pltpu.make_async_copy(w2_hbm.at[D:F], w2_v.at[D:F], sem_in.at[9])
    cp_go = pltpu.make_async_copy(go_hbm, go_raw, sem_in.at[4])
    cp_wq = pltpu.make_async_copy(wq_hbm, wq_ref, sem_in.at[6])
    cp_wo = pltpu.make_async_copy(wo_hbm, wo_ref, sem_in.at[7])
    cp_dwq = pltpu.make_async_copy(wq_ref, dwq_hbm, sem_out.at[6])
    cp_dwo = pltpu.make_async_copy(wo_ref, dwo_hbm, sem_out.at[7])

    def cp_out(i):
        return pltpu.make_async_copy(go_raw.at[_tile(i, LT), :], out_hbm.at[_tile(i, LT), :], sem_out.at[0])

    def cp_dw2(i):
        return pltpu.make_async_copy(w2_v.at[:, _tile(i, LT)], dw2_hbm.at[:, _tile(i, LT)], sem_out.at[1])

    def cp_dw1(i):
        return pltpu.make_async_copy(w1_v.at[:, _tile(i, LT)], dw1_hbm.at[:, _tile(i, LT)], sem_out.at[2])

    def cp_dx(i):
        return pltpu.make_async_copy(x_raw.at[_tile(i, LT), :], dx_hbm.at[_tile(i, LT), :], sem_out.at[3])

    cvec = c_ref[...].astype(F32)
    csig = jax.nn.sigmoid(cvec)
    sc = cvec * csig
    wkvT = jnp.concatenate([wk_ref[...], wv_ref[...]], axis=0)
    z8 = jnp.zeros((8, LT), F32)
    inv_d = 1.0 / D

    def pipeline(n, mm, ew, bufs, lo=0):
        mm(lo, bufs[0])

        def body(j, carry):
            i = lo + 2 * j
            ew(i, bufs[0])
            mm(i + 1, bufs[1])
            ew(i + 1, bufs[1])
            mm(i + 2, bufs[0])
            return carry
        lax.fori_loop(0, (n - lo) // 2 - 1, body, 0)
        ew(n - 2, bufs[0])
        mm(n - 1, bufs[1])
        ew(n - 1, bufs[1])

    def scope1(wmod_v, kv_s, xb, h1a, h1b, qn_s, hb, l0, l1):
        def mod_parts(lo, hi):
            mod = _dot(jnp.broadcast_to(sc, (16, D)).astype(BF16), wmod_v[:, lo * D:hi * D])[0:1]
            modrow[:, lo * D:hi * D] = mod
            for r in range(lo, hi):
                m_r = mod[:, (r - lo) * D:(r - lo + 1) * D]
                if r in (1, 4):
                    m_r = m_r + 1.0
                modc[r] = jnp.broadcast_to(m_r, (LT, D)).T

        with _scope("P1"):
            cp_wma = pltpu.make_async_copy(wmod_hbm.at[:, 0:2 * D], wmod_v.at[:, 0:2 * D], sem_in.at[1])
            cp_wmb = pltpu.make_async_copy(wmod_hbm.at[:, 2 * D:6 * D], wmod_v.at[:, 2 * D:6 * D], sem_in.at[5])
            cp_wma.start()
            cp_xa.start()
            cp_wq.start()
            cp_xb.start()
            b1v[...] = b1_ref[...].astype(F32).reshape(1, F)
            b2v[...] = b2_ref[...].astype(F32).reshape(1, S)
            qn_s[...] = jnp.zeros(qn_s.shape, F32)
            cp_wma.wait()
            mod_parts(0, 2)
            cp_wq.wait()
            wqT_s[...] = _pk(wq_ref[...].T)

        with _scope("P2"):
            cp_xa.wait()
            cp_wmb.start()
            cp_wo.start()
            cp_go.start()

            def ln1_chunk(i, hbuf):
                tl = _tile(i, LT)
                for rs in _blocks(D, LT):
                    xb[rs, :] = x_raw[tl, rs].T.astype(F32)
                c = xb[0:1, :]
                s1 = s2 = z8
                for rs in _blocks(D, RB):
                    d = xb[rs, :] - c
                    s1 = s1 + _bsum(d)
                    s2 = s2 + _bsum(d * d)
                mu, r = _moments(s1, s2, c)
                st[0:1, tl] = mu
                st[1:2, tl] = r
                for rs in _blocks(D, RB):
                    h1 = _pk((((xb[rs, :] - mu) * r) * modc[1, rs] + modc[0, rs]).astype(BF16))
                    hbuf[_pr(rs.start, RB), :] = h1
                    h1T[_pr(rs.start, RB), tl] = h1

            def proj_chunk(i, hbuf):
                tl = _tile(i, LT)
                h1 = _up(hbuf[...])
                kv_s[:, tl] = _dot(wkvT, h1)
                for m in range(0, D, 256):
                    q = (_dot(_up(wqT_s[_pr(m, 256), :]), h1) * QSCALE).astype(BF16)
                    q3 = q.reshape(256 // DH, DH, LT)
                    hs = slice(m // DH, (m + 256) // DH)
                    QA[hs, 0:DH, tl] = q3
                    QA[hs, DH:AR, tl] = jnp.zeros((256 // DH, AR - DH, LT), BF16)
                    qf = q3.astype(F32)
                    qn_s[...] = jnp.maximum(qn_s[...], jnp.max(jnp.sum(qf * qf, axis=1), axis=0, keepdims=True))

            pipeline(NLT // 2, ln1_chunk, proj_chunk, (h1a, h1b))
            cp_xb.wait()
            pipeline(NLT, ln1_chunk, proj_chunk, (h1a, h1b), lo=NLT // 2)

        with _scope("P3"):
            kvT = kv_s[...]
            kTb = kvT[0:DH].astype(BF16)
            vTb = kvT[DH:2 * DH].astype(BF16)
            KT[...] = kTb
            VT[...] = vTb
            rows = lax.broadcasted_iota(jnp.int32, (LT - DH, S), 0)
            tail = jnp.where(rows < 3, 1.0, 0.0).astype(BF16)
            ka_t = jnp.concatenate([kTb, tail], axis=0)
            va_t = jnp.concatenate([vTb, tail], axis=0)
            for j in range(NLT):
                KA[_pr(j * LT, LT), :] = _pk(ka_t[:, j * LT:(j + 1) * LT].T)
                VA[_pr(j * LT, LT), :] = _pk(va_t[:, j * LT:(j + 1) * LT].T)

            kf = kTb.astype(F32)
            kn2 = jnp.max(jnp.sum(kf * kf, axis=0, keepdims=True))
            bound2 = jnp.max(qn_s[...]) * kn2
            vmax = jnp.max(jnp.abs(vTb.astype(F32)))
            safe = jnp.logical_and(bound2 <= SAFE_BOUND * SAFE_BOUND, vmax <= 1e15)

            cp_wmb.wait()
            mod_parts(2, 6)
            cp_wo.wait()
            woT_s[...] = _pk(wo_ref[...].T)
            cp_go.wait()

        def keys(ref, lo, n):
            return _up(ref[_pr(lo, n), :])[:, 0:AR]

        with _scope("P4max"):
            @pl.when(jnp.logical_not(safe))
            def _():
                def pmax(t, carry):
                    h = t // NQ
                    q = QA[h, :, _lanes(t)]
                    m = None
                    for lo in range(0, S, KC_F):
                        mc = jnp.max(_dot(keys(KA, lo, KC_F), q), axis=0, keepdims=True)
                        m = mc if m is None else jnp.maximum(m, mc)
                    hi, mid, lo_ = _split3(m)
                    QA[h, DH:AR, _lanes(t)] = _rows16((-hi, -mid, -lo_), (AR - DH, W), 0)
                    return carry
                lax.fori_loop(0, NT, pmax, 0)

        def p_out(idx):
            return pltpu.make_async_copy(hb.at[idx % 4], p_hbm.at[idx], sem_p.at[idx % 4])

        def fwd_step(t_next, pn, ln, t_cur, pc, lc):
            q = QA[t_next // NQ, :, _lanes(t_next)]
            lacc = jnp.zeros((32, W), F32)
            o = jnp.zeros((DH, W), F32)
            for c in range(S // KC_F):
                for lo in range(c * KC_F, (c + 1) * KC_F, SUB_F):
                    p = jnp.exp2(_dot(keys(KA, lo, SUB_F), q))
                    pn[_pr(lo, SUB_F), :] = _pk(p.astype(BF16))
                    lacc = lacc + p.reshape(SUB_F // 32, 32, W).sum(axis=0)
                if t_cur is not None:
                    for lo in range(c * KC_F, (c + 1) * KC_F, 128):
                        o = o + _dot(VT[:, lo:lo + 128], _up(pc[_pr(lo, 128), :]))
            lnew = lacc.sum(axis=0, keepdims=True)
            if t_cur is not None:
                hc = t_cur // NQ
                linv = 1.0 / lc[...]
                oT[pl.ds(pl.multiple_of(hc * (DH // 2), DH // 2), DH // 2), _lanes(t_cur)] = _pk(
                    (o * linv).astype(BF16))
                sh = QA[hc, DH:AR, _lanes(t_cur)].astype(F32)
                hi, mid, lo = _split3(linv)
                QA[hc, DH:AR, _lanes(t_cur)] = _rows16(
                    (sh[0:1], sh[1:2], sh[2:3], hi, mid, lo), (AR - DH, W), 0)
            ln[...] = lnew

        with _scope("P4"):
            fwd_step(0, hb.at[0], l0, None, None, None)
            p_out(0).start()

            def fwd_body(it, carry):
                t = 4 * it
                pv = pres.at[it]
                ha = hb.at[(2 * it) % 4]
                hc = hb.at[(2 * it + 1) % 4]
                hn = hb.at[(2 * it + 2) % 4]
                p0 = pres2.at[_slot0(it)]

                @pl.when(it >= 2)
                def _():
                    p_out(2 * it - 3).wait()

                @pl.when(it >= 1)
                def _():
                    p_out(2 * it - 2).wait()
                goT[_tile(it % 4, LT // 2), _tile(it // 4, LT)] = _pk(
                    go_raw[_tile(it // 4, LT), _tile(it % 4, LT)].T)
                fwd_step(t + 1, pv, l1, t, ha, l0)
                fwd_step(t + 2, hc, l0, t + 1, pv, l1)
                p_out(2 * it + 1).start()
                fwd_step(t + 3, p0, l1, t + 2, hc, l0)
                fwd_step(jnp.minimum(t + 4, NT - 1), hn, l0, t + 3, p0, l1)

                @pl.when(it + 1 < NIT)
                def _():
                    p_out(2 * it + 2).start()
                return carry
            lax.fori_loop(0, NIT, fwd_body, 0)
            cp_w2a.start()
            cp_w2b.start()
            cp_w1.start()
            for k in range(3):
                p_out(2 * NIT - 3 + k).wait()

    pl.run_scoped(scope1, V((D, 6 * D), BF16), V((2 * DH, S), F32), V((D, LT), F32),
                  V((D // 2, LT), U32), V((D // 2, LT), U32), V((1, LT), F32),
                  V((4, S // 2, W), U32),
                  V((1, W), F32), V((1, W), F32))

    def scope2(x1T, h3T, g_s, gT_s, du_s, duT_s, dgbuf, ta, tb, tc, td):
        def a_mm(i, abuf):
            och = _up(oT[:, _tile(i, LT)])
            for m in range(0, D, 256):
                abuf[m:m + 256, :] = _dot(_up(woT_s[_pr(m, 256), :]), och)

        def dg_mm(sl):
            w2r = w2_v[sl, :]
            for m in range(0, D, 256):
                dgbuf[m:m + 256, sl] = _dot_nt(_up(goT[_pr(m, 256), :]), w2r)

        def p5_ew(i, abuf):
            tl = _tile(i, LT)
            for rs in _blocks(D, LT):
                x1T[rs, tl] = x_raw[tl, rs].T.astype(F32) + modc[2, rs] * abuf[rs, :]
            c = x1T[0:1, tl]
            s1 = s2 = z8
            for rs in _blocks(D, RB):
                d = x1T[rs, tl] - c
                s1 = s1 + _bsum(d)
                s2 = s2 + _bsum(d * d)
            mu2, r2 = _moments(s1, s2, c)

            def h2_of(rs):
                return ((x1T[rs, tl] - mu2) * r2) * modc[4, rs] + modc[3, rs]
            c3 = h2_of(slice(0, 8))[0:1]
            s1 = s2 = z8
            for rs in _blocks(D, RB):
                d = h2_of(rs) - c3
                s1 = s1 + _bsum(d)
                s2 = s2 + _bsum(d * d)
            mu3, r3 = _moments(s1, s2, c3)
            st[2:3, tl] = mu2
            st[3:4, tl] = r2
            st[4:5, tl] = mu3
            st[5:6, tl] = r3
            for rs in _blocks(D, RB):
                h3T[_pr(rs.start, RB), tl] = _pk(((h2_of(rs) - mu3) * r3).astype(BF16))

        with _scope("P5"):
            a_mm(0, ta)

            def p5a(j, carry):
                i = 2 * j
                p5_ew(i, ta)
                a_mm(i + 1, tb)
                p5_ew(i + 1, tb)
                a_mm(i + 2, ta)
                return carry
            lax.fori_loop(0, 2, p5a, 0)
            p5_ew(4, ta)
            a_mm(5, tb)
            p5_ew(5, tb)
            a_mm(6, ta)

            def p5b(j, carry):
                i = 6 + 2 * j
                p5_ew(i, ta)
                a_mm(i + 1, tb)
                dg_mm(_tile(2 * j, 128))
                p5_ew(i + 1, tb)
                a_mm(jnp.minimum(i + 2, NLT - 1), ta)
                dg_mm(_tile(2 * j + 1, 128))
                return carry
            cp_w2a.wait()
            lax.fori_loop(0, 2, p5b, 0)
            cp_w2b.wait()
            lax.fori_loop(2, NFC // 2, p5b, 0)
            dg_mm(slice(NFC * 128, F))

        def u_mm(sl, n, ubuf):
            w1r = w1_v[sl, :]
            for m in range(0, D, 256):
                ubuf[m:m + 256, 0:n] = _dot_nt(_up(h3T[_pr(m, 256), :]), w1r)

        def f_ew(sl, sl2, n, ubuf):
            b1r = b1v[:, sl]
            sdb = jnp.zeros((8, n), F32)
            for rs in _blocks(D, LT):
                gb = modc[5, rs, 0:n]
                u = ubuf[rs, 0:n] + b1r
                u2 = u * u
                t = jnp.tanh(C0 * u * (1.0 + C1 * u2))
                hp = 0.5 * (1.0 + t)
                g = u * hp
                du = (dgbuf[rs, sl] * gb) * (hp + 0.5 * u * (1.0 - t * t) * C0 * (1.0 + 3.0 * C1 * u2))
                dub = du.astype(BF16)
                g_s[_pr(rs.start, LT), sl] = _pk(g.astype(BF16))
                du_s[_pr(rs.start, LT), sl] = _pk(dub)
                gT_s[sl2, rs] = _pk((g * gb).astype(BF16).T)
                duT_s[sl2, rs] = _pk(dub.T)
                sdb = sdb + _bsum(du)
            db1v[:, sl] = _fin(sdb)

        with _scope("P6"):
            cp_w1.wait()
            u_mm(slice(0, 128), 128, ta)

            def p6(j, carry):
                i = 2 * j
                f_ew(_tile(i, 128), _tile(i, 64), 128, ta)
                u_mm(_tile(i + 1, 128), 128, tb)
                f_ew(_tile(i + 1, 128), _tile(i + 1, 64), 128, tb)
                u_mm(_tile(i + 2, 128), 128, ta)
                return carry
            lax.fori_loop(0, NFC // 2 - 1, p6, 0)
            i8, i9 = NFC - 2, NFC - 1
            f_ew(slice(i8 * 128, i9 * 128), slice(i8 * 64, i9 * 64), 128, ta)
            u_mm(slice(i9 * 128, NFC * 128), 128, tb)
            f_ew(slice(i9 * 128, NFC * 128), slice(i9 * 64, NFC * 64), 128, tb)
            u_mm(slice(NFC * 128, F), FT, ta)
            f_ew(slice(NFC * 128, F), slice(NFC * 64, F // 2), FT, ta)

        def p7_mm(i, bufs):
            yb, hb_ = bufs
            tl = _tile(i, LT)
            w2c = w2_v[:, tl]
            w1c = w1_v[:, tl]
            for m in range(0, D, MB):
                yb[m:m + MB, :] = _dot(_up(g_s[_pr(m, MB), :]), w2c)
            for m in range(0, D, MB):
                hb_[m:m + MB, :] = _dot(_up(du_s[_pr(m, MB), :]), w1c)
            goc = _up(goT[:, tl])
            h3c = _up(h3T[:, tl])
            for rs in _blocks(F, MB):
                w2_v[rs, tl] = _dot(_up(gT_s[_pr(rs.start, rs.stop - rs.start), :]), goc).astype(BF16)
            for rs in _blocks(F, MB):
                w1_v[rs, tl] = _dot(_up(duT_s[_pr(rs.start, rs.stop - rs.start), :]), h3c).astype(BF16)
            cp_dw2(i).start()
            cp_dw1(i).start()

        def p7_ew(i, bufs):
            yb, hb_ = bufs
            tl = _tile(i, LT)
            b2r = b2v[:, tl]
            mu2, r2, mu3, r3 = st[2:3, tl], st[3:4, tl], st[4:5, tl], st[5:6, tl]
            for rs in _blocks(D, LT):
                go_raw[tl, rs] = (x1T[rs, tl] + modc[5, rs] * (yb[rs, :] + b2r)).astype(BF16).T
            cp_out(i).start()

            def norms(rs):
                n2 = (x1T[rs, tl] - mu2) * r2
                h3 = (n2 * modc[4, rs] + modc[3, rs] - mu3) * r3
                return n2, h3

            def dx2_of(rs):
                return _up(goT[_pr(rs.start, RB), tl]).astype(F32)

            s1 = s2 = sdb = z8
            for rs in _blocks(D, RB):
                dx2 = dx2_of(rs)
                acc_s[5, rs] += dx2 * (yb[rs, :] + b2r)
                sdb = sdb + _bsum(modc[5, rs] * dx2)
                _, h3 = norms(rs)
                dh3 = hb_[rs, :]
                s1 = s1 + _bsum(dh3)
                s2 = s2 + _bsum(dh3 * h3)
            db2v[:, tl] = _fin(sdb)
            m1 = _fin(s1) * inv_d
            m2 = _fin(s2) * inv_d
            s3 = s4 = z8
            for rs in _blocks(D, RB):
                n2, h3 = norms(rs)
                dh2 = r3 * (hb_[rs, :] - m1 - h3 * m2)
                acc_s[4, rs] += dh2 * n2
                acc_s[3, rs] += dh2
                dn2 = dh2 * modc[4, rs]
                hb_[rs, :] = dn2
                s3 = s3 + _bsum(dn2)
                s4 = s4 + _bsum(dn2 * n2)
            m3 = _fin(s3) * inv_d
            m4 = _fin(s4) * inv_d
            for rs in _blocks(D, RB):
                n2 = (x1T[rs, tl] - mu2) * r2
                dx1 = dx2_of(rs) + r2 * (hb_[rs, :] - m3 - n2 * m4)
                dx1b[_pr(rs.start, RB), tl] = _pk(dx1.astype(BF16))

        with _scope("P7"):
            acc_s[...] = jnp.zeros(acc_s.shape, F32)
            pipeline(NLT, p7_mm, p7_ew, ((ta, tb), (tc, td)))

        db1_ref[...] = db1v[...].reshape(F).astype(BF16)
        db2_ref[...] = db2v[...].reshape(S).astype(BF16)
        for r in (3, 4, 5):
            dmod_s[:, r * D:(r + 1) * D] = _row_of(acc_s[r])

    pl.run_scoped(scope2, V((D, S), F32), V((D // 2, S), U32), V((D // 2, F), U32),
                  V((F // 2, D), U32), V((D // 2, F), U32), V((F // 2, D), U32),
                  V((D, F), F32),
                  V((D, LT), F32), V((D, LT), F32), V((D, LT), F32), V((D, LT), F32))

    def scope3(DOA, dqT, dkT, dvT, wm, dsc_s, hb):
        def p_in(idx):
            return pltpu.make_async_copy(p_hbm.at[jnp.minimum(idx, 2 * NIT - 1)], hb.at[idx % 4],
                                         sem_p.at[idx % 4])

        cp_wm = pltpu.make_async_copy(wmod_hbm, wm, sem_in.at[1])
        cp_dwm_b = pltpu.make_async_copy(wm.at[:, 2 * D:6 * D], dwmod_hbm.at[:, 2 * D:6 * D], sem_out.at[4])
        cp_dwm_a = pltpu.make_async_copy(wm.at[:, 0:2 * D], dwmod_hbm.at[:, 0:2 * D], sem_out.at[5])
        sc_col = jnp.broadcast_to(sc, (LT, D)).T

        def mod_bwd(lo, hi):
            dm = dmod_s[:, lo * D:hi * D]
            part = _dot_nt(jnp.broadcast_to(dm, (16, (hi - lo) * D)).astype(BF16), wm[:, lo * D:hi * D])[0:1]
            for j in range(lo * D // LT, hi * D // LT):
                wm[:, j * LT:(j + 1) * LT] = (sc_col * dmod_s[:, j * LT:(j + 1) * LT]).astype(BF16)
            return part

        def scope_p8(wog, m_acc, ta, tb):
            def p8_mm(i, dbuf_):
                tl = _tile(i, LT)
                dxc = _up(dx1b[:, tl])
                for m in range(0, D, 256):
                    dbuf_[m:m + 256, :] = _dot(_up(wog[_pr(m, 256), :]), dxc)
                for m in range(0, D, 256):
                    m_acc[m:m + 256, :] += _dot_nt(_up(oT[_pr(m, 256), tl]), dxc)

            def p8_ew(i, dbuf_):
                tl = _tile(i, LT)
                hpb = RB // DH
                for rs in _blocks(D, RB):
                    hs = slice(rs.start // DH, rs.stop // DH)
                    li = QA[hs, DH:AR, tl].astype(F32)
                    linv = li[:, 3:4] + li[:, 4:5] + li[:, 5:6]
                    dos = (dbuf_[rs, :].reshape(hpb, DH, LT) * linv).astype(BF16)
                    of = _up(oT[_pr(rs.start, RB), tl]).astype(F32).reshape(hpb, DH, LT)
                    delta = jnp.sum(dos.astype(F32) * of, axis=1, keepdims=True)
                    hi, mid, lo = _split3(delta)
                    DOA[hs, 0:DH, tl] = dos
                    DOA[hs, DH:AR, tl] = _rows16((-hi, -mid, -lo), (hpb, AR - DH, LT), 1)

            garow = modrow[:, 2 * D:3 * D]
            wof = wo_ref[...].astype(F32)
            wog[...] = _pk((wof * garow).astype(BF16))
            m_acc[...] = jnp.zeros(m_acc.shape, F32)
            pipeline(NLT, p8_mm, p8_ew, (ta, tb))
            m_od = m_acc[...]
            dmod_s[:, 2 * D:3 * D] = jnp.sum(m_od * wo_ref[...].astype(F32), axis=0, keepdims=True)
            wo_ref[...] = (m_od * garow).astype(BF16)
            cp_dwo.start()
            cp_wm.wait()
            dsc_s[...] = mod_bwd(2, 6)
            cp_dwm_b.start()

        with _scope("P8"):
            cp_wm.start()
            p_in(0).start()
            p_in(1).start()
            p_in(2).start()
            pl.run_scoped(scope_p8, V((D // 2, D), U32), V((D, D), F32), V((D, LT), F32), V((D, LT), F32))

        def scope_p9(db0, db1):
            def keys(ref, lo, n):
                return _up(ref[_pr(lo, n), :])[:, 0:AR]

            def bwd_step(t_next, pn, dn, recompute, t_cur, pc, dc):
                hn = t_next // NQ
                if recompute:
                    qa = QA[hn, :, _lanes(t_next)]
                doa = DOA[hn, :, _lanes(t_next)]
                if t_cur is not None:
                    hc = t_cur // NQ
                    qt = QA[hc, 0:DH, _lanes(t_cur)]
                    dot_ = DOA[hc, 0:DH, _lanes(t_cur)]
                    dq = jnp.zeros((DH, W), F32)

                def stage1(lo):
                    if recompute:
                        s = _dot(keys(KA, lo, SUB_B), qa)
                    dp = _dot(keys(VA, lo, SUB_B), doa)
                    if recompute:
                        p = jnp.exp2(s)
                        pn[_pr(lo, SUB_B), :] = _pk(p.astype(BF16))
                    else:
                        p = _up(pn[_pr(lo, SUB_B), :]).astype(F32)
                    dn[_pr(lo, SUB_B), :] = _pk((p * dp).astype(BF16))

                half = KC_B // 2
                for c in range(S // KC_B):
                    sl = slice(c * KC_B, (c + 1) * KC_B)
                    for lo in range(c * KC_B, c * KC_B + half, SUB_B):
                        stage1(lo)
                    if t_cur is not None:
                        ds = _up(dc[_pr(c * KC_B, KC_B), :])
                        dkT[:, sl] += _dot_nt(qt, ds)
                    for lo in range(c * KC_B + half, (c + 1) * KC_B, SUB_B):
                        stage1(lo)
                    if t_cur is not None:
                        dvT[:, sl] += _dot_nt(dot_, _up(pc[_pr(c * KC_B, KC_B), :]))
                        dq = dq + _dot(KT[:, sl], ds)
                if t_cur is not None:
                    dqT[pl.ds(pl.multiple_of(hc * (DH // 2), DH // 2), DH // 2), _lanes(t_cur)] = _pk(
                        (dq * 0.25).astype(BF16))

            dkT[...] = jnp.zeros(dkT.shape, F32)
            dvT[...] = jnp.zeros(dvT.shape, F32)
            p_in(0).wait()
            bwd_step(0, hb.at[0], db0, False, None, None, None)

            def bwd_body(recompute, it, carry):
                t = 4 * it
                pv = pres.at[it]
                ha = hb.at[(2 * it) % 4]
                hc = hb.at[(2 * it + 1) % 4]
                hn = hb.at[(2 * it + 2) % 4]
                p0 = pres2.at[_slot0(it)]
                p_in(2 * it + 1).wait()
                p_in(2 * it + 2).wait()
                p_in(2 * it + 3).start()
                bwd_step(t + 1, pv, db1, False, t, ha, db0)
                p_in(2 * it + 4).start()
                bwd_step(t + 2, hc, db0, False, t + 1, pv, db1)
                bwd_step(t + 3, p0, db1, recompute, t + 2, hc, db0)
                bwd_step(jnp.minimum(t + 4, NT - 1), hn, db0, False, t + 3, p0, db1)
                return carry
            lax.fori_loop(0, NIT - NV2, functools.partial(bwd_body, True), 0)
            lax.fori_loop(NIT - NV2, NIT, functools.partial(bwd_body, False), 0)
            p_in(2 * NIT + 1).wait()
            p_in(2 * NIT + 2).wait()

        with _scope("P9"):
            pl.run_scoped(scope_p9, V((S // 2, W), U32), V((S // 2, W), U32))

        def scope_p10(dkv_s, dwq_acc, wqp, ta, tb, nb):
            def p10_mm(i, hbuf):
                tl = _tile(i, LT)
                dqc = _up(dqT[:, tl])
                kvc = dkv_s[:, tl]
                for m in range(0, D, 256):
                    hbuf[m:m + 256, :] = _dot(_up(wqp[_pr(m, 256), :]), dqc) + _dot(wkv_n[m:m + 256], kvc)
                for m in range(0, D, 256):
                    dwq_acc[m:m + 256, :] += _dot_nt(_up(h1T[_pr(m, 256), tl]), dqc)

            def p10_ew(i, hbuf):
                tl = _tile(i, LT)
                mu, r = st[0:1, tl], st[1:2, tl]
                for rs in _blocks(D, LT):
                    nb[rs, :] = (x_raw[tl, rs].T.astype(F32) - mu) * r
                s1 = s2 = z8
                for rs in _blocks(D, RB):
                    dh1 = hbuf[rs, :]
                    n1 = nb[rs, :]
                    acc_s[1, rs] += dh1 * n1
                    acc_s[0, rs] += dh1
                    dn1 = dh1 * modc[1, rs]
                    hbuf[rs, :] = dn1
                    s1 = s1 + _bsum(dn1)
                    s2 = s2 + _bsum(dn1 * n1)
                m1 = _fin(s1) * inv_d
                m2 = _fin(s2) * inv_d
                for rs in _blocks(D, LT):
                    dx1 = _up(dx1b[_pr(rs.start, LT), tl]).astype(F32)
                    dx0 = dx1 + r * (hbuf[rs, :] - m1 - nb[rs, :] * m2)
                    x_raw[tl, rs] = dx0.astype(BF16).T
                cp_dx(i).start()

            dkv = jnp.concatenate([dkT[...] * LN2, dvT[...]], axis=0).astype(BF16)
            dkv_s[...] = dkv
            wkv_n = wkvT.T
            wqp[...] = _pk(wq_ref[...])
            dwq_acc[...] = jnp.zeros(dwq_acc.shape, F32)
            pipeline(NLT, p10_mm, p10_ew, (ta, tb))
            wq_ref[...] = dwq_acc[...].astype(BF16)
            cp_dwq.start()
            dwkvT = _dot_nt(dkv_s[...], _up(h1T[...]))
            dwk_ref[...] = dwkvT[0:DH].astype(BF16)
            dwv_ref[...] = dwkvT[DH:2 * DH].astype(BF16)

        with _scope("P10"):
            pl.run_scoped(scope_p10, V((2 * DH, S), BF16), V((D, D), F32), V((D // 2, D), U32),
                          V((D, LT), F32), V((D, LT), F32), V((D, LT), F32))

        with _scope("P11"):
            for r in (0, 1):
                dmod_s[:, r * D:(r + 1) * D] = _row_of(acc_s[r])
            dsc = dsc_s[...] + mod_bwd(0, 2)
            cp_dwm_a.start()
            dc_ref[...] = (dsc * (csig * (1.0 + cvec * (1.0 - csig)))).astype(BF16)
            for i in range(NLT):
                cp_out(i).wait()
                cp_dw2(i).wait()
                cp_dw1(i).wait()
                cp_dx(i).wait()
            cp_dwo.wait()
            cp_dwq.wait()
            cp_dwm_b.wait()
            cp_dwm_a.wait()

    pl.run_scoped(scope3, V((H, AR, S), BF16), V((D // 2, S), U32), V((DH, S), F32), V((DH, S), F32),
                  V((D, 6 * D), BF16), V((1, D), F32), V((4, S // 2, W), U32))


@jax.jit
def pallas_adaLN_cond__grouped_kv_mqa__mixer_token_mlp__prompt_kernel(
    A_x: jax.Array,
    A_wq: jax.Array,
    A_wk: jax.Array,
    A_wv: jax.Array,
    A_wo: jax.Array,
    B_x: jax.Array,
    B_w1: jax.Array,
    B_b1: jax.Array,
    B_w2: jax.Array,
    B_b2: jax.Array,
    c: jax.Array,
    w_mod: jax.Array,
    grad_out: jax.Array,
):
    del B_x
    any_spec = pl.BlockSpec(memory_space=pl.ANY)
    vmem_spec = pl.BlockSpec(memory_space=pltpu.VMEM)
    sds = jax.ShapeDtypeStruct
    out_shape = (
        sds((S, D), BF16), sds((S, D), BF16),
        sds((D, D), BF16), sds((DH, D), BF16), sds((DH, D), BF16), sds((D, D), BF16),
        sds((F, S), BF16), sds((F,), BF16), sds((F, S), BF16), sds((S,), BF16),
        sds((1, D), BF16), sds((D, 6 * D), BF16),
        sds((2 * NIT, S // 2, W), U32),
    )
    in_specs = [any_spec, any_spec, vmem_spec, vmem_spec, any_spec, any_spec, vmem_spec, any_spec,
                vmem_spec, vmem_spec, any_spec, any_spec]
    out_specs = (any_spec, any_spec, any_spec, vmem_spec, vmem_spec, any_spec, any_spec, vmem_spec,
                 any_spec, vmem_spec, vmem_spec, any_spec, any_spec)
    V = pltpu.VMEM
    scratch = [
        V((NIT, S // 2, W), U32), V((NV2 + 1, S // 2, W), U32),
        V((H, AR, S), BF16),
        V((S // 2, LT), U32), V((S // 2, LT), U32), V((DH, S), BF16), V((DH, S), BF16),
        V((S, D), BF16), V((S, D), BF16), V((F, S), BF16), V((F, S), BF16),
        V((D // 2, S), U32), V((D // 2, S), U32), V((D // 2, S), U32),
        V((D // 2, S), U32), V((8, S), F32),
        V((6, D, LT), F32), V((1, 6 * D), F32), V((6, D, LT), F32),
        V((D, D), BF16), V((D, D), BF16),
        V((D // 2, D), U32), V((D // 2, D), U32), V((1, F), F32), V((1, S), F32),
        V((1, F), F32), V((1, S), F32), V((1, 6 * D), F32),
        pltpu.SemaphoreType.DMA((10,)), pltpu.SemaphoreType.DMA((8,)), pltpu.SemaphoreType.DMA((4,)),
    ]
    res = pl.pallas_call(
        _kernel,
        out_shape=out_shape,
        in_specs=in_specs,
        out_specs=out_specs,
        scratch_shapes=scratch,
        compiler_params=pltpu.CompilerParams(vmem_limit_bytes=127 * 1024 * 1024),
    )(A_x.reshape(S, D), A_wq, A_wk.T, A_wv.T, A_wo, B_w1.T, B_b1, B_w2, B_b2,
      c, w_mod, grad_out.reshape(S, D))
    (out, dx, dwq, dwk, dwv, dwo, dw1, db1, dw2, db2, dc, dwmod, _) = res
    return (out.reshape(1, S, D), dx.reshape(1, S, D), dwq, dwk.T, dwv.T, dwo, dw1.T, db1, dw2,
            db2, dc, dwmod)
```

```python
import contextlib
import functools

import jax
import jax.numpy as jnp
from jax import lax
import jax.experimental.pallas as pl
import jax.experimental.pallas.tpu as pltpu

S, D, H, DH, F = 2048, 512, 32, 16, 1376
EPS = 1e-5
LOG2E = 1.4426950408889634
LN2 = 0.6931471805599453
QSCALE = 0.25 * LOG2E
C0 = 0.7978845608028654
C1 = 0.044715

LT = 128
NLT = S // LT
W = 256
NQ = S // W
NT = H * NQ
NIT = NT // 4
NV2 = 10
NRB = 8
KC_F = 512
SUB_F = 256
KC_B = 256
SUB_B = 64
MB = 256
RB = 64
AR = 32
NFC = F // 128
FT = F % 128
SAFE_BOUND = 40.0

_PROFILE = False


def _scope(name):
    return jax.named_scope(name) if _PROFILE else contextlib.nullcontext()


F32 = jnp.float32
BF16 = jnp.bfloat16
U32 = jnp.uint32
NT_DIMS = (((1,), (1,)), ((), ()))


def _dot(a, b):
    return jnp.dot(a, b, preferred_element_type=F32)


def _dot_nt(a, b):
    return lax.dot_general(a, b, NT_DIMS, preferred_element_type=F32)


def _tile(i, n):
    return pl.ds(pl.multiple_of(i * n, n), n)


def _pk(x):
    return pltpu.bitcast(x, U32)


def _up(x):
    return pltpu.bitcast(x, BF16)


def _pr(m, n):
    return slice(m // 2, (m + n) // 2)


def _split3(x):
    hi = x.astype(BF16).astype(F32)
    r = x - hi
    mid = r.astype(BF16).astype(F32)
    lo = (r - mid).astype(BF16).astype(F32)
    return hi, mid, lo


def _rows16(vals, shape, axis):
    row = lax.broadcasted_iota(jnp.int32, shape, axis)
    blk = jnp.zeros(shape, F32)
    for k, v in enumerate(vals):
        blk = jnp.where(row == k, v, blk)
    return blk.astype(BF16)


def _bsum(x):
    return x.reshape(x.shape[0] // 8, 8, x.shape[1]).sum(axis=0)


def _fin(s8):
    return jnp.sum(s8, axis=0, keepdims=True)


def _moments(s1, s2, c):
    d = _fin(s1) * (1.0 / D)
    var = jnp.maximum(_fin(s2) * (1.0 / D) - d * d, 0.0)
    return c + d, lax.rsqrt(var + EPS)


def _row_of(acc):
    return jnp.sum(acc.T, axis=0, keepdims=True)


def _lanes(t):
    return pl.ds(pl.multiple_of((t % NQ) * W, W), W)


def _slot0(it):
    return jnp.maximum(it - (NIT - NV2 - 1), 0)


def _blocks(n, step):
    return [slice(m, min(m + step, n)) for m in range(0, n, step)]


def _kernel(
    x_hbm, wq_hbm, wk_ref, wv_ref, wo_hbm, w1_hbm, b1_ref, w2_hbm, b2_ref, c_ref, wmod_hbm, go_hbm,
    out_hbm, dx_hbm, dwq_hbm, dwk_ref, dwv_ref, dwo_hbm, dw1_hbm, db1_ref, dw2_hbm, db2_ref, dc_ref, dwmod_hbm,
    p_hbm,
    pres, pres2, QA, KA, VA, KT, VT, x_raw, go_raw, w1_v, w2_v, oT, h1T, goT, dx1b, st, modrow,
    wq_ref, wo_ref, b1v, b2v, db1v, db2v, dmod_s,
    sem_in, sem_out, sem_p,
):
    V = pltpu.VMEM
    cp_xa = pltpu.make_async_copy(x_hbm.at[0:S // 2], x_raw.at[0:S // 2], sem_in.at[0])
    cp_xb = pltpu.make_async_copy(x_hbm.at[S // 2:S], x_raw.at[S // 2:S], sem_in.at[8])
    cp_w1 = pltpu.make_async_copy(w1_hbm, w1_v, sem_in.at[2])
    cp_w2a = pltpu.make_async_copy(w2_hbm.at[0:D], w2_v.at[0:D], sem_in.at[3])
    cp_w2b = pltpu.make_async_copy(w2_hbm.at[D:F], w2_v.at[D:F], sem_in.at[9])
    cp_go = pltpu.make_async_copy(go_hbm, go_raw, sem_in.at[4])
    cp_wq = pltpu.make_async_copy(wq_hbm, wq_ref, sem_in.at[6])
    cp_wo = pltpu.make_async_copy(wo_hbm, wo_ref, sem_in.at[7])
    cp_dwq = pltpu.make_async_copy(wq_ref, dwq_hbm, sem_out.at[6])
    cp_dwo = pltpu.make_async_copy(wo_ref, dwo_hbm, sem_out.at[7])

    def cp_out(i):
        return pltpu.make_async_copy(go_raw.at[_tile(i, LT), :], out_hbm.at[_tile(i, LT), :], sem_out.at[0])

    def cp_dw2(i):
        return pltpu.make_async_copy(w2_v.at[:, _tile(i, LT)], dw2_hbm.at[:, _tile(i, LT)], sem_out.at[1])

    def cp_dw1(i):
        return pltpu.make_async_copy(w1_v.at[:, _tile(i, LT)], dw1_hbm.at[:, _tile(i, LT)], sem_out.at[2])

    def cp_dx(i):
        return pltpu.make_async_copy(x_raw.at[_tile(i, LT), :], dx_hbm.at[_tile(i, LT), :], sem_out.at[3])

    cvec = c_ref[...].astype(F32)
    csig = jax.nn.sigmoid(cvec)
    sc = cvec * csig
    wkvT = jnp.concatenate([wk_ref[...], wv_ref[...]], axis=0)
    z8 = jnp.zeros((8, LT), F32)
    inv_d = 1.0 / D

    def mod_col(r):
        m_r = modrow[:, r * D:(r + 1) * D]
        if r in (1, 4):
            m_r = m_r + 1.0
        return jnp.broadcast_to(m_r, (LT, D)).T

    def pipeline(n, mm, ew, bufs, lo=0):
        mm(lo, bufs[0])

        def body(j, carry):
            i = lo + 2 * j
            ew(i, bufs[0])
            mm(i + 1, bufs[1])
            ew(i + 1, bufs[1])
            mm(i + 2, bufs[0])
            return carry
        lax.fori_loop(0, (n - lo) // 2 - 1, body, 0)
        ew(n - 2, bufs[0])
        mm(n - 1, bufs[1])
        ew(n - 1, bufs[1])

    def scope1(wmod_v, kv_s, xb, h1a, h1b, qn_s, hb, l0, l1, modc, wqT_s):
        def mod_parts(lo, hi):
            modrow[:, lo * D:hi * D] = _dot(
                jnp.broadcast_to(sc, (16, D)).astype(BF16), wmod_v[:, lo * D:hi * D])[0:1]

        with _scope("P1"):
            cp_wma = pltpu.make_async_copy(wmod_hbm.at[:, 0:2 * D], wmod_v.at[:, 0:2 * D], sem_in.at[1])
            cp_wmb = pltpu.make_async_copy(wmod_hbm.at[:, 2 * D:6 * D], wmod_v.at[:, 2 * D:6 * D], sem_in.at[5])
            cp_wma.start()
            cp_xa.start()
            cp_wq.start()
            cp_xb.start()
            b1v[...] = b1_ref[...].astype(F32).reshape(1, F)
            b2v[...] = b2_ref[...].astype(F32).reshape(1, S)
            qn_s[...] = jnp.zeros(qn_s.shape, F32)
            cp_wma.wait()
            mod_parts(0, 2)
            modc[0] = mod_col(0)
            modc[1] = mod_col(1)
            cp_wq.wait()
            wqT_s[...] = _pk(wq_ref[...].T)

        with _scope("P2"):
            cp_xa.wait()
            cp_wmb.start()
            cp_wo.start()
            cp_go.start()

            def ln1_chunk(i, hbuf):
                tl = _tile(i, LT)
                for rs in _blocks(D, LT):
                    xb[rs, :] = x_raw[tl, rs].T.astype(F32)
                c = xb[0:1, :]
                s1 = s2 = z8
                for rs in _blocks(D, RB):
                    d = xb[rs, :] - c
                    s1 = s1 + _bsum(d)
                    s2 = s2 + _bsum(d * d)
                mu, r = _moments(s1, s2, c)
                st[0:1, tl] = mu
                st[1:2, tl] = r
                for rs in _blocks(D, RB):
                    h1 = _pk((((xb[rs, :] - mu) * r) * modc[1, rs] + modc[0, rs]).astype(BF16))
                    hbuf[_pr(rs.start, RB), :] = h1
                    h1T[_pr(rs.start, RB), tl] = h1

            def proj_chunk(i, hbuf):
                tl = _tile(i, LT)
                h1 = _up(hbuf[...])
                kv_s[:, tl] = _dot(wkvT, h1)
                for m in range(0, D, 256):
                    q = (_dot(_up(wqT_s[_pr(m, 256), :]), h1) * QSCALE).astype(BF16)
                    q3 = q.reshape(256 // DH, DH, LT)
                    hs = slice(m // DH, (m + 256) // DH)
                    QA[hs, 0:DH, tl] = q3
                    QA[hs, DH:AR, tl] = jnp.zeros((256 // DH, AR - DH, LT), BF16)
                    qf = q3.astype(F32)
                    qn_s[...] = jnp.maximum(qn_s[...], jnp.max(jnp.sum(qf * qf, axis=1), axis=0, keepdims=True))

            pipeline(NLT // 2, ln1_chunk, proj_chunk, (h1a, h1b))
            cp_xb.wait()
            pipeline(NLT, ln1_chunk, proj_chunk, (h1a, h1b), lo=NLT // 2)

        with _scope("P3"):
            kvT = kv_s[...]
            kTb = kvT[0:DH].astype(BF16)
            vTb = kvT[DH:2 * DH].astype(BF16)
            KT[...] = kTb
            VT[...] = vTb
            rows = lax.broadcasted_iota(jnp.int32, (LT - DH, S), 0)
            tail = jnp.where(rows < 3, 1.0, 0.0).astype(BF16)
            ka_t = jnp.concatenate([kTb, tail], axis=0)
            va_t = jnp.concatenate([vTb, tail], axis=0)
            for j in range(NLT):
                KA[_pr(j * LT, LT), :] = _pk(ka_t[:, j * LT:(j + 1) * LT].T)
                VA[_pr(j * LT, LT), :] = _pk(va_t[:, j * LT:(j + 1) * LT].T)

            kf = kTb.astype(F32)
            kn2 = jnp.max(jnp.sum(kf * kf, axis=0, keepdims=True))
            bound2 = jnp.max(qn_s[...]) * kn2
            vmax = jnp.max(jnp.abs(vTb.astype(F32)))
            safe = jnp.logical_and(bound2 <= SAFE_BOUND * SAFE_BOUND, vmax <= 1e15)

            cp_wmb.wait()
            mod_parts(2, 6)
            cp_wo.wait()
            cp_go.wait()

        def keys(ref, lo, n):
            return _up(ref[_pr(lo, n), :])[:, 0:AR]

        with _scope("P4max"):
            @pl.when(jnp.logical_not(safe))
            def _():
                def pmax(t, carry):
                    h = t // NQ
                    q = QA[h, :, _lanes(t)]
                    m = None
                    for lo in range(0, S, KC_F):
                        mc = jnp.max(_dot(keys(KA, lo, KC_F), q), axis=0, keepdims=True)
                        m = mc if m is None else jnp.maximum(m, mc)
                    hi, mid, lo_ = _split3(m)
                    QA[h, DH:AR, _lanes(t)] = _rows16((-hi, -mid, -lo_), (AR - DH, W), 0)
                    return carry
                lax.fori_loop(0, NT, pmax, 0)

        def p_out(idx):
            return pltpu.make_async_copy(hb.at[idx % 4], p_hbm.at[idx], sem_p.at[idx % 4])

        def fwd_step(t_next, pn, ln, t_cur, pc, lc):
            q = QA[t_next // NQ, :, _lanes(t_next)]
            lacc = jnp.zeros((32, W), F32)
            o = jnp.zeros((DH, W), F32)
            for c in range(S // KC_F):
                for lo in range(c * KC_F, (c + 1) * KC_F, SUB_F):
                    p = jnp.exp2(_dot(keys(KA, lo, SUB_F), q))
                    pn[_pr(lo, SUB_F), :] = _pk(p.astype(BF16))
                    lacc = lacc + p.reshape(SUB_F // 32, 32, W).sum(axis=0)
                if t_cur is not None:
                    for lo in range(c * KC_F, (c + 1) * KC_F, 128):
                        o = o + _dot(VT[:, lo:lo + 128], _up(pc[_pr(lo, 128), :]))
            lnew = lacc.sum(axis=0, keepdims=True)
            if t_cur is not None:
                hc = t_cur // NQ
                linv = 1.0 / lc[...]
                oT[pl.ds(pl.multiple_of(hc * (DH // 2), DH // 2), DH // 2), _lanes(t_cur)] = _pk(
                    (o * linv).astype(BF16))
                sh = QA[hc, DH:AR, _lanes(t_cur)].astype(F32)
                hi, mid, lo = _split3(linv)
                QA[hc, DH:AR, _lanes(t_cur)] = _rows16(
                    (sh[0:1], sh[1:2], sh[2:3], hi, mid, lo), (AR - DH, W), 0)
            ln[...] = lnew

        with _scope("P4"):
            fwd_step(0, hb.at[0], l0, None, None, None)
            p_out(0).start()

            def fwd_body(it, carry):
                t = 4 * it
                pv = pres.at[it]
                ha = hb.at[(2 * it) % 4]
                hc = hb.at[(2 * it + 1) % 4]
                hn = hb.at[(2 * it + 2) % 4]
                p0 = pres2.at[_slot0(it)]

                @pl.when(it >= 2)
                def _():
                    p_out(2 * it - 3).wait()

                @pl.when(it >= 1)
                def _():
                    p_out(2 * it - 2).wait()
                goT[_tile(it % 4, LT // 2), _tile(it // 4, LT)] = _pk(
                    go_raw[_tile(it // 4, LT), _tile(it % 4, LT)].T)
                fwd_step(t + 1, pv, l1, t, ha, l0)
                fwd_step(t + 2, hc, l0, t + 1, pv, l1)
                p_out(2 * it + 1).start()
                fwd_step(t + 3, p0, l1, t + 2, hc, l0)
                fwd_step(jnp.minimum(t + 4, NT - 1), hn, l0, t + 3, p0, l1)

                @pl.when(it + 1 < NIT)
                def _():
                    p_out(2 * it + 2).start()
                return carry
            lax.fori_loop(0, NIT, fwd_body, 0)
            cp_w2a.start()
            cp_w2b.start()
            cp_w1.start()
            for k in range(3):
                p_out(2 * NIT - 3 + k).wait()

    pl.run_scoped(scope1, V((D, 6 * D), BF16), V((2 * DH, S), F32), V((D, LT), F32),
                  V((D // 2, LT), U32), V((D // 2, LT), U32), V((1, LT), F32),
                  V((4, S // 2, W), U32),
                  V((1, W), F32), V((1, W), F32), V((2, D, LT), F32), V((D // 2, D), U32))

    def scope2(x1T, h3T, g_s, gT_s, du_s, duT_s, dgbuf, ta, tb, tc, td, modc, acc_s, woT_s):
        def a_mm(i, abuf):
            och = _up(oT[:, _tile(i, LT)])
            for m in range(0, D, 256):
                abuf[m:m + 256, :] = _dot(_up(woT_s[_pr(m, 256), :]), och)

        def dg_mm(sl):
            w2r = w2_v[sl, :]
            for m in range(0, D, 256):
                dgbuf[m:m + 256, sl] = _dot_nt(_up(goT[_pr(m, 256), :]), w2r)

        def p5_ew(i, abuf):
            tl = _tile(i, LT)
            for rs in _blocks(D, LT):
                x1T[rs, tl] = x_raw[tl, rs].T.astype(F32) + modc[0, rs] * abuf[rs, :]
            c = x1T[0:1, tl]
            s1 = s2 = z8
            for rs in _blocks(D, RB):
                d = x1T[rs, tl] - c
                s1 = s1 + _bsum(d)
                s2 = s2 + _bsum(d * d)
            mu2, r2 = _moments(s1, s2, c)

            def h2_of(rs):
                return ((x1T[rs, tl] - mu2) * r2) * modc[2, rs] + modc[1, rs]
            c3 = h2_of(slice(0, 8))[0:1]
            s1 = s2 = z8
            for rs in _blocks(D, RB):
                d = h2_of(rs) - c3
                s1 = s1 + _bsum(d)
                s2 = s2 + _bsum(d * d)
            mu3, r3 = _moments(s1, s2, c3)
            st[2:3, tl] = mu2
            st[3:4, tl] = r2
            st[4:5, tl] = mu3
            st[5:6, tl] = r3
            for rs in _blocks(D, RB):
                h3T[_pr(rs.start, RB), tl] = _pk(((h2_of(rs) - mu3) * r3).astype(BF16))

        with _scope("P5"):
            woT_s[...] = _pk(wo_ref[...].T)
            for r in range(4):
                modc[r] = mod_col(r + 2)
            a_mm(0, ta)

            def p5a(j, carry):
                i = 2 * j
                p5_ew(i, ta)
                a_mm(i + 1, tb)
                p5_ew(i + 1, tb)
                a_mm(i + 2, ta)
                return carry
            lax.fori_loop(0, 2, p5a, 0)
            p5_ew(4, ta)
            a_mm(5, tb)
            p5_ew(5, tb)
            a_mm(6, ta)

            def p5b(j, carry):
                i = 6 + 2 * j
                p5_ew(i, ta)
                a_mm(i + 1, tb)
                dg_mm(_tile(2 * j, 128))
                p5_ew(i + 1, tb)
                a_mm(jnp.minimum(i + 2, NLT - 1), ta)
                dg_mm(_tile(2 * j + 1, 128))
                return carry
            cp_w2a.wait()
            lax.fori_loop(0, 2, p5b, 0)
            cp_w2b.wait()
            lax.fori_loop(2, NFC // 2, p5b, 0)
            dg_mm(slice(NFC * 128, F))

        def u_mm(sl, n, ubuf):
            w1r = w1_v[sl, :]
            for m in range(0, D, 256):
                ubuf[m:m + 256, 0:n] = _dot_nt(_up(h3T[_pr(m, 256), :]), w1r)

        def f_ew(sl, sl2, n, ubuf):
            b1r = b1v[:, sl]
            sdb = jnp.zeros((8, n), F32)
            for rs in _blocks(D, LT):
                gb = modc[3, rs, 0:n]
                u = ubuf[rs, 0:n] + b1r
                u2 = u * u
                t = jnp.tanh(C0 * u * (1.0 + C1 * u2))
                hp = 0.5 * (1.0 + t)
                g = u * hp
                du = (dgbuf[rs, sl] * gb) * (hp + 0.5 * u * (1.0 - t * t) * C0 * (1.0 + 3.0 * C1 * u2))
                dub = du.astype(BF16)
                g_s[_pr(rs.start, LT), sl] = _pk(g.astype(BF16))
                du_s[_pr(rs.start, LT), sl] = _pk(dub)
                gT_s[sl2, rs] = _pk((g * gb).astype(BF16).T)
                duT_s[sl2, rs] = _pk(dub.T)
                sdb = sdb + _bsum(du)
            db1v[:, sl] = _fin(sdb)

        with _scope("P6"):
            cp_w1.wait()
            u_mm(slice(0, 128), 128, ta)

            def p6(j, carry):
                i = 2 * j
                f_ew(_tile(i, 128), _tile(i, 64), 128, ta)
                u_mm(_tile(i + 1, 128), 128, tb)
                f_ew(_tile(i + 1, 128), _tile(i + 1, 64), 128, tb)
                u_mm(_tile(i + 2, 128), 128, ta)
                return carry
            lax.fori_loop(0, NFC // 2 - 1, p6, 0)
            i8, i9 = NFC - 2, NFC - 1
            f_ew(slice(i8 * 128, i9 * 128), slice(i8 * 64, i9 * 64), 128, ta)
            u_mm(slice(i9 * 128, NFC * 128), 128, tb)
            f_ew(slice(i9 * 128, NFC * 128), slice(i9 * 64, NFC * 64), 128, tb)
            u_mm(slice(NFC * 128, F), FT, ta)
            f_ew(slice(NFC * 128, F), slice(NFC * 64, F // 2), FT, ta)

        def p7_mm(i, bufs):
            yb, hb_ = bufs
            tl = _tile(i, LT)
            w2c = w2_v[:, tl]
            w1c = w1_v[:, tl]
            for m in range(0, D, MB):
                yb[m:m + MB, :] = _dot(_up(g_s[_pr(m, MB), :]), w2c)
            for m in range(0, D, MB):
                hb_[m:m + MB, :] = _dot(_up(du_s[_pr(m, MB), :]), w1c)
            goc = _up(goT[:, tl])
            h3c = _up(h3T[:, tl])
            for rs in _blocks(F, MB):
                w2_v[rs, tl] = _dot(_up(gT_s[_pr(rs.start, rs.stop - rs.start), :]), goc).astype(BF16)
            for rs in _blocks(F, MB):
                w1_v[rs, tl] = _dot(_up(duT_s[_pr(rs.start, rs.stop - rs.start), :]), h3c).astype(BF16)
            cp_dw2(i).start()
            cp_dw1(i).start()

        def p7_ew(i, bufs):
            yb, hb_ = bufs
            tl = _tile(i, LT)
            b2r = b2v[:, tl]
            mu2, r2, mu3, r3 = st[2:3, tl], st[3:4, tl], st[4:5, tl], st[5:6, tl]
            for rs in _blocks(D, LT):
                go_raw[tl, rs] = (x1T[rs, tl] + modc[3, rs] * (yb[rs, :] + b2r)).astype(BF16).T
            cp_out(i).start()

            def norms(rs):
                n2 = (x1T[rs, tl] - mu2) * r2
                h3 = (n2 * modc[2, rs] + modc[1, rs] - mu3) * r3
                return n2, h3

            def dx2_of(rs):
                return _up(goT[_pr(rs.start, RB), tl]).astype(F32)

            s1 = s2 = sdb = z8
            for rs in _blocks(D, RB):
                dx2 = dx2_of(rs)
                acc_s[2, rs] += dx2 * (yb[rs, :] + b2r)
                sdb = sdb + _bsum(modc[3, rs] * dx2)
                _, h3 = norms(rs)
                dh3 = hb_[rs, :]
                s1 = s1 + _bsum(dh3)
                s2 = s2 + _bsum(dh3 * h3)
            db2v[:, tl] = _fin(sdb)
            m1 = _fin(s1) * inv_d
            m2 = _fin(s2) * inv_d
            s3 = s4 = z8
            for rs in _blocks(D, RB):
                n2, h3 = norms(rs)
                dh2 = r3 * (hb_[rs, :] - m1 - h3 * m2)
                acc_s[1, rs] += dh2 * n2
                acc_s[0, rs] += dh2
                dn2 = dh2 * modc[2, rs]
                hb_[rs, :] = dn2
                s3 = s3 + _bsum(dn2)
                s4 = s4 + _bsum(dn2 * n2)
            m3 = _fin(s3) * inv_d
            m4 = _fin(s4) * inv_d
            for rs in _blocks(D, RB):
                n2 = (x1T[rs, tl] - mu2) * r2
                dx1 = dx2_of(rs) + r2 * (hb_[rs, :] - m3 - n2 * m4)
                dx1b[_pr(rs.start, RB), tl] = _pk(dx1.astype(BF16))

        with _scope("P7"):
            acc_s[...] = jnp.zeros(acc_s.shape, F32)
            pipeline(NLT, p7_mm, p7_ew, ((ta, tb), (tc, td)))

        db1_ref[...] = db1v[...].reshape(F).astype(BF16)
        db2_ref[...] = db2v[...].reshape(S).astype(BF16)
        for r in (3, 4, 5):
            dmod_s[:, r * D:(r + 1) * D] = _row_of(acc_s[r - 3])

    pl.run_scoped(scope2, V((D, S), F32), V((D // 2, S), U32), V((D // 2, F), U32),
                  V((F // 2, D), U32), V((D // 2, F), U32), V((F // 2, D), U32),
                  V((D, F), F32),
                  V((D, LT), F32), V((D, LT), F32), V((D, LT), F32), V((D, LT), F32),
                  V((4, D, LT), F32), V((3, D, LT), F32), V((D // 2, D), U32))

    def scope3(DOA, dqT, dkT, dvT, wm, dsc_s, hb):
        def p_in(idx):
            return pltpu.make_async_copy(p_hbm.at[jnp.minimum(idx, 2 * NIT - 1)], hb.at[idx % NRB],
                                         sem_p.at[idx % NRB])

        cp_wm = pltpu.make_async_copy(wmod_hbm, wm, sem_in.at[1])
        cp_dwm_b = pltpu.make_async_copy(wm.at[:, 2 * D:6 * D], dwmod_hbm.at[:, 2 * D:6 * D], sem_out.at[4])
        cp_dwm_a = pltpu.make_async_copy(wm.at[:, 0:2 * D], dwmod_hbm.at[:, 0:2 * D], sem_out.at[5])
        sc_col = jnp.broadcast_to(sc, (LT, D)).T

        def mod_bwd(lo, hi):
            dm = dmod_s[:, lo * D:hi * D]
            part = _dot_nt(jnp.broadcast_to(dm, (16, (hi - lo) * D)).astype(BF16), wm[:, lo * D:hi * D])[0:1]
            for j in range(lo * D // LT, hi * D // LT):
                wm[:, j * LT:(j + 1) * LT] = (sc_col * dmod_s[:, j * LT:(j + 1) * LT]).astype(BF16)
            return part

        def scope_p8(wog, m_acc, ta, tb):
            def p8_mm(i, dbuf_):
                tl = _tile(i, LT)
                dxc = _up(dx1b[:, tl])
                for m in range(0, D, 256):
                    dbuf_[m:m + 256, :] = _dot(_up(wog[_pr(m, 256), :]), dxc)
                for m in range(0, D, 256):
                    m_acc[m:m + 256, :] += _dot_nt(_up(oT[_pr(m, 256), tl]), dxc)

            def p8_ew(i, dbuf_):
                tl = _tile(i, LT)
                hpb = RB // DH
                for rs in _blocks(D, RB):
                    hs = slice(rs.start // DH, rs.stop // DH)
                    li = QA[hs, DH:AR, tl].astype(F32)
                    linv = li[:, 3:4] + li[:, 4:5] + li[:, 5:6]
                    dos = (dbuf_[rs, :].reshape(hpb, DH, LT) * linv).astype(BF16)
                    of = _up(oT[_pr(rs.start, RB), tl]).astype(F32).reshape(hpb, DH, LT)
                    delta = jnp.sum(dos.astype(F32) * of, axis=1, keepdims=True)
                    hi, mid, lo = _split3(delta)
                    DOA[hs, 0:DH, tl] = dos
                    DOA[hs, DH:AR, tl] = _rows16((-hi, -mid, -lo), (hpb, AR - DH, LT), 1)

            garow = modrow[:, 2 * D:3 * D]
            wof = wo_ref[...].astype(F32)
            wog[...] = _pk((wof * garow).astype(BF16))
            m_acc[...] = jnp.zeros(m_acc.shape, F32)
            pipeline(NLT, p8_mm, p8_ew, (ta, tb))
            m_od = m_acc[...]
            dmod_s[:, 2 * D:3 * D] = jnp.sum(m_od * wo_ref[...].astype(F32), axis=0, keepdims=True)
            wo_ref[...] = (m_od * garow).astype(BF16)
            cp_dwo.start()
            cp_wm.wait()
            dsc_s[...] = mod_bwd(2, 6)
            cp_dwm_b.start()

        with _scope("P8"):
            cp_wm.start()
            for k in range(5):
                p_in(k).start()
            pl.run_scoped(scope_p8, V((D // 2, D), U32), V((D, D), F32), V((D, LT), F32), V((D, LT), F32))

        def scope_p9(db0, db1):
            def keys(ref, lo, n):
                return _up(ref[_pr(lo, n), :])[:, 0:AR]

            def bwd_step(t_next, pn, dn, recompute, t_cur, pc, dc):
                hn = t_next // NQ
                if recompute:
                    qa = QA[hn, :, _lanes(t_next)]
                doa = DOA[hn, :, _lanes(t_next)]
                if t_cur is not None:
                    hc = t_cur // NQ
                    qt = QA[hc, 0:DH, _lanes(t_cur)]
                    dot_ = DOA[hc, 0:DH, _lanes(t_cur)]
                    dq = jnp.zeros((DH, W), F32)

                def stage1(lo):
                    if recompute:
                        s = _dot(keys(KA, lo, SUB_B), qa)
                    dp = _dot(keys(VA, lo, SUB_B), doa)
                    if recompute:
                        p = jnp.exp2(s)
                        pn[_pr(lo, SUB_B), :] = _pk(p.astype(BF16))
                    else:
                        p = _up(pn[_pr(lo, SUB_B), :]).astype(F32)
                    dn[_pr(lo, SUB_B), :] = _pk((p * dp).astype(BF16))

                half = KC_B // 2
                for c in range(S // KC_B):
                    sl = slice(c * KC_B, (c + 1) * KC_B)
                    for lo in range(c * KC_B, c * KC_B + half, SUB_B):
                        stage1(lo)
                    if t_cur is not None:
                        ds = _up(dc[_pr(c * KC_B, KC_B), :])
                        dkT[:, sl] += _dot_nt(qt, ds)
                    for lo in range(c * KC_B + half, (c + 1) * KC_B, SUB_B):
                        stage1(lo)
                    if t_cur is not None:
                        dvT[:, sl] += _dot_nt(dot_, _up(pc[_pr(c * KC_B, KC_B), :]))
                        dq = dq + _dot(KT[:, sl], ds)
                if t_cur is not None:
                    dqT[pl.ds(pl.multiple_of(hc * (DH // 2), DH // 2), DH // 2), _lanes(t_cur)] = _pk(
                        (dq * 0.25).astype(BF16))

            dkT[...] = jnp.zeros(dkT.shape, F32)
            dvT[...] = jnp.zeros(dvT.shape, F32)
            p_in(0).wait()
            bwd_step(0, hb.at[0], db0, False, None, None, None)

            def bwd_body(recompute, j, carry):
                for k in range(1, 5):
                    p_in(4 * j + k).wait()
                for k in range(5, 8):
                    p_in(4 * j + k).start()
                for g in range(2):
                    it = 2 * j + g
                    t = 4 * it
                    pv = pres.at[it]
                    ha = hb.at[(2 * it) % NRB]
                    hc = hb.at[(2 * it + 1) % NRB]
                    hn = hb.at[(2 * it + 2) % NRB]
                    p0 = pres2.at[_slot0(it)]
                    bwd_step(t + 1, pv, db1, False, t, ha, db0)
                    if g == 0:
                        p_in(4 * j + 8).start()
                    bwd_step(t + 2, hc, db0, False, t + 1, pv, db1)
                    bwd_step(t + 3, p0, db1, recompute, t + 2, hc, db0)
                    bwd_step(jnp.minimum(t + 4, NT - 1), hn, db0, False, t + 3, p0, db1)
                return carry
            lax.fori_loop(0, (NIT - NV2) // 2, functools.partial(bwd_body, True), 0)
            lax.fori_loop((NIT - NV2) // 2, NIT // 2, functools.partial(bwd_body, False), 0)
            for k in range(1, 5):
                p_in(2 * NIT + k).wait()

        with _scope("P9"):
            pl.run_scoped(scope_p9, V((S // 2, W), U32), V((S // 2, W), U32))

        def scope_p10(dkv_s, dwq_acc, wqp, ta, tb, nb, ca1, acc_s):
            def p10_mm(i, hbuf):
                tl = _tile(i, LT)
                dqc = _up(dqT[:, tl])
                kvc = dkv_s[:, tl]
                for m in range(0, D, 256):
                    hbuf[m:m + 256, :] = _dot(_up(wqp[_pr(m, 256), :]), dqc) + _dot(wkv_n[m:m + 256], kvc)
                for m in range(0, D, 256):
                    dwq_acc[m:m + 256, :] += _dot_nt(_up(h1T[_pr(m, 256), tl]), dqc)

            def p10_ew(i, hbuf):
                tl = _tile(i, LT)
                mu, r = st[0:1, tl], st[1:2, tl]
                for rs in _blocks(D, LT):
                    nb[rs, :] = (x_raw[tl, rs].T.astype(F32) - mu) * r
                s1 = s2 = z8
                for rs in _blocks(D, RB):
                    dh1 = hbuf[rs, :]
                    n1 = nb[rs, :]
                    acc_s[1, rs] += dh1 * n1
                    acc_s[0, rs] += dh1
                    dn1 = dh1 * ca1[rs]
                    hbuf[rs, :] = dn1
                    s1 = s1 + _bsum(dn1)
                    s2 = s2 + _bsum(dn1 * n1)
                m1 = _fin(s1) * inv_d
                m2 = _fin(s2) * inv_d
                for rs in _blocks(D, LT):
                    dx1 = _up(dx1b[_pr(rs.start, LT), tl]).astype(F32)
                    dx0 = dx1 + r * (hbuf[rs, :] - m1 - nb[rs, :] * m2)
                    x_raw[tl, rs] = dx0.astype(BF16).T
                cp_dx(i).start()

            dkv = jnp.concatenate([dkT[...] * LN2, dvT[...]], axis=0).astype(BF16)
            dkv_s[...] = dkv
            wkv_n = wkvT.T
            wqp[...] = _pk(wq_ref[...])
            dwq_acc[...] = jnp.zeros(dwq_acc.shape, F32)
            acc_s[...] = jnp.zeros(acc_s.shape, F32)
            ca1[...] = mod_col(1)
            pipeline(NLT, p10_mm, p10_ew, (ta, tb))
            for r in (0, 1):
                dmod_s[:, r * D:(r + 1) * D] = _row_of(acc_s[r])
            wq_ref[...] = dwq_acc[...].astype(BF16)
            cp_dwq.start()
            dwkvT = _dot_nt(dkv_s[...], _up(h1T[...]))
            dwk_ref[...] = dwkvT[0:DH].astype(BF16)
            dwv_ref[...] = dwkvT[DH:2 * DH].astype(BF16)

        with _scope("P10"):
            pl.run_scoped(scope_p10, V((2 * DH, S), BF16), V((D, D), F32), V((D // 2, D), U32),
                          V((D, LT), F32), V((D, LT), F32), V((D, LT), F32),
                          V((D, LT), F32), V((2, D, LT), F32))

        with _scope("P11"):
            dsc = dsc_s[...] + mod_bwd(0, 2)
            cp_dwm_a.start()
            dc_ref[...] = (dsc * (csig * (1.0 + cvec * (1.0 - csig)))).astype(BF16)
            for i in range(NLT):
                cp_out(i).wait()
                cp_dw2(i).wait()
                cp_dw1(i).wait()
                cp_dx(i).wait()
            cp_dwo.wait()
            cp_dwq.wait()
            cp_dwm_b.wait()
            cp_dwm_a.wait()

    pl.run_scoped(scope3, V((H, AR, S), BF16), V((D // 2, S), U32), V((DH, S), F32), V((DH, S), F32),
                  V((D, 6 * D), BF16), V((1, D), F32), V((NRB, S // 2, W), U32))


@jax.jit
def pallas_adaLN_cond__grouped_kv_mqa__mixer_token_mlp__prompt_kernel(
    A_x: jax.Array,
    A_wq: jax.Array,
    A_wk: jax.Array,
    A_wv: jax.Array,
    A_wo: jax.Array,
    B_x: jax.Array,
    B_w1: jax.Array,
    B_b1: jax.Array,
    B_w2: jax.Array,
    B_b2: jax.Array,
    c: jax.Array,
    w_mod: jax.Array,
    grad_out: jax.Array,
):
    del B_x
    any_spec = pl.BlockSpec(memory_space=pl.ANY)
    vmem_spec = pl.BlockSpec(memory_space=pltpu.VMEM)
    sds = jax.ShapeDtypeStruct
    out_shape = (
        sds((S, D), BF16), sds((S, D), BF16),
        sds((D, D), BF16), sds((DH, D), BF16), sds((DH, D), BF16), sds((D, D), BF16),
        sds((F, S), BF16), sds((F,), BF16), sds((F, S), BF16), sds((S,), BF16),
        sds((1, D), BF16), sds((D, 6 * D), BF16),
        sds((2 * NIT, S // 2, W), U32),
    )
    in_specs = [any_spec, any_spec, vmem_spec, vmem_spec, any_spec, any_spec, vmem_spec, any_spec,
                vmem_spec, vmem_spec, any_spec, any_spec]
    out_specs = (any_spec, any_spec, any_spec, vmem_spec, vmem_spec, any_spec, any_spec, vmem_spec,
                 any_spec, vmem_spec, vmem_spec, any_spec, any_spec)
    V = pltpu.VMEM
    scratch = [
        V((NIT, S // 2, W), U32), V((NV2 + 1, S // 2, W), U32),
        V((H, AR, S), BF16),
        V((S // 2, LT), U32), V((S // 2, LT), U32), V((DH, S), BF16), V((DH, S), BF16),
        V((S, D), BF16), V((S, D), BF16), V((F, S), BF16), V((F, S), BF16),
        V((D // 2, S), U32), V((D // 2, S), U32), V((D // 2, S), U32),
        V((D // 2, S), U32), V((8, S), F32),
        V((1, 6 * D), F32),
        V((D, D), BF16), V((D, D), BF16),
        V((1, F), F32), V((1, S), F32),
        V((1, F), F32), V((1, S), F32), V((1, 6 * D), F32),
        pltpu.SemaphoreType.DMA((10,)), pltpu.SemaphoreType.DMA((8,)), pltpu.SemaphoreType.DMA((NRB,)),
    ]
    res = pl.pallas_call(
        _kernel,
        out_shape=out_shape,
        in_specs=in_specs,
        out_specs=out_specs,
        scratch_shapes=scratch,
        compiler_params=pltpu.CompilerParams(vmem_limit_bytes=127 * 1024 * 1024),
    )(A_x.reshape(S, D), A_wq, A_wk.T, A_wv.T, A_wo, B_w1.T, B_b1, B_w2, B_b2,
      c, w_mod, grad_out.reshape(S, D))
    (out, dx, dwq, dwk, dwv, dwo, dw1, db1, dw2, db2, dc, dwmod, _) = res
    return (out.reshape(1, S, D), dx.reshape(1, S, D), dwq, dwk.T, dwv.T, dwo, dw1.T, db1, dw2,
            db2, dc, dwmod)
```
